```python
import jax
import jax.numpy as jnp

def _softmax(x, axis=-1):
    return jax.nn.softmax(x, axis=axis)

def _gelu(x):
    return jax.nn.gelu(x, approximate=True)

def _silu(x):
    return jax.nn.silu(x)

def _sigmoid(x):
    return jax.nn.sigmoid(x)

def _layernorm(x, axis=-1, eps=1e-05):
    m = jnp.mean(x, axis=axis, keepdims=True)
    v = jnp.var(x, axis=axis, keepdims=True)
    return (x - m) / jnp.sqrt(v + eps)

def _scatter_add(tgt, idx, src, axis=0):
    return tgt.at[idx].add(src)

def _segment_sum(src, seg, n):
    return jax.ops.segment_sum(src, seg, n)

class _Rng:

    def __init__(self, key):
        self._k = key

    def _next(self):
        self._k, sub = jax.random.split(self._k)
        return sub

    def normal(self, shape):
        return jax.random.normal(self._next(), shape, dtype=jnp.bfloat16)

    def randint(self, lo, hi, shape):
        return jax.random.randint(self._next(), shape, lo, hi, dtype=jnp.int32)

    def uniform(self, shape, lo=0.0, hi=1.0):
        return jax.random.uniform(self._next(), shape, jnp.bfloat16, lo, hi)

    def permutation(self, n):
        return jax.random.permutation(self._next(), n)
kernel_name = 'interleave_layers__memory_aug_recurrent_mem_tr__glu_gated_glu__prompt'

def setup_inputs():
    _rng = _Rng(jax.random.key(int.from_bytes(__import__("os").urandom(4), "little")))
    _w = lambda a: (lambda t: t.astype(jnp.bfloat16) if jnp.issubdtype(t.dtype, jnp.floating) else t)(jnp.asarray(a))

    def _A_setup():
        B, S, Dm = (1, 2048, 1024)
        H, Dh = (32, 128)
        M, seg = (8, 32)
        seg = min(seg, S)
        S = S // seg * seg
        return {'x': _w((lambda *s: _rng.normal(s) * 0.05)(B, S, Dm)), 'mem0': _w((lambda *s: _rng.normal(s) * 0.05)(B, M, Dm)), 'Wq': _w((lambda *s: _rng.normal(s) * 0.05)(Dm, H, Dh) * Dm ** (-0.5)), 'Wk': _w((lambda *s: _rng.normal(s) * 0.05)(Dm, H, Dh) * Dm ** (-0.5)), 'Wv': _w((lambda *s: _rng.normal(s) * 0.05)(Dm, H, Dh) * Dm ** (-0.5)), 'Wo': _w((lambda *s: _rng.normal(s) * 0.05)(H, Dh, Dm) * (H * Dh) ** (-0.5)), 'seg_len': seg}
    _A_in = _A_setup()

    def _B_setup():
        B, S, D, F = (1, 2048, 1024, 3584)
        return {'x': _w((lambda *s: _rng.normal(s) * 0.05)(B, S, D)), 'w_gate': _w((lambda *s: _rng.normal(s) * 0.05)(D, F)), 'w_up': _w((lambda *s: _rng.normal(s) * 0.05)(D, F)), 'w_down': _w((lambda *s: _rng.normal(s) * 0.05)(F, D))}
    _B_in = _B_setup()
    return {'A_x': _A_in['x'], 'A_mem0': _A_in['mem0'], 'A_Wq': _A_in['Wq'], 'A_Wk': _A_in['Wk'], 'A_Wv': _A_in['Wv'], 'A_Wo': _A_in['Wo'], 'A_seg_len': _A_in['seg_len'], 'B_x': _B_in['x'], 'B_w_gate': _B_in['w_gate'], 'B_w_up': _B_in['w_up'], 'B_w_down': _B_in['w_down']}

def reference(A_x, A_mem0, A_Wq, A_Wk, A_Wv, A_Wo, A_seg_len, B_x, B_w_gate, B_w_up, B_w_down):

    def _A_ref(x, mem0, Wq, Wk, Wv, Wo, seg_len):
        B, S, Dm = x.shape
        H, Dh = (Wq.shape[1], Wq.shape[2])
        M = mem0.shape[1]
        scale = Dh ** (-0.5)
        n_seg = S // seg_len
        L = M + seg_len
        idx = jnp.arange(L)
        mask = (idx[:, None] < M) | (idx[:, None] >= idx[None, :])
        mem = mem0
        outs = []
        for s in range(n_seg):
            xs = x[:, s * seg_len:(s + 1) * seg_len, :].copy()
            h = jnp.concatenate([mem, xs], axis=1)
            q = jnp.einsum('btd,dhe->bhte', h, Wq)
            k = jnp.einsum('btd,dhe->bhte', h, Wk)
            v = jnp.einsum('btd,dhe->bhte', h, Wv)
            scores = jnp.einsum('bhqe,bhke->bhqk', q, k) * scale
            scores = jnp.where(mask[None, None], scores, -1000000000.0)
            p = _softmax(scores, axis=-1)
            o = jnp.einsum('bhqk,bhke->bhqe', p, v)
            o = jnp.einsum('bhte,hed->btd', o, Wo)
            mem = o[:, :M, :].copy()
            outs.append(o[:, M:, :])
        return jnp.concatenate(outs, axis=1)

    def _B_ref(x, w_gate, w_up, w_down):
        g = jnp.einsum('bsd,df->bsf', x, w_gate)
        u = jnp.einsum('bsd,df->bsf', x, w_up)
        h = _sigmoid(g) * u
        return jnp.einsum('bsf,fd->bsd', h, w_down)
    x = A_x
    x = x + _A_ref(_layernorm(x, axis=-1), A_mem0, A_Wq, A_Wk, A_Wv, A_Wo, A_seg_len)
    x = x + _B_ref(_layernorm(x, axis=-1), B_w_gate, B_w_up, B_w_down)
    x = x + _A_ref(_layernorm(x, axis=-1), A_mem0, A_Wq, A_Wk, A_Wv, A_Wo, A_seg_len)
    x = x + _B_ref(_layernorm(x, axis=-1), B_w_gate, B_w_up, B_w_down)
    return x
```

```python
import functools
import jax
import jax.numpy as jnp
from jax import lax
from jax.experimental import pallas as pl
from jax.experimental.pallas import tpu as pltpu

S, DM, H, DH, M, SEG, FF = 2048, 1024, 32, 128, 8, 32, 3584
NSEG = S // SEG
MP = 2 * M
U32 = jnp.uint32
BF16 = jnp.bfloat16
F32 = jnp.float32
EPS = 1e-5
NEG = -1e9
LOG2E = 1.4426950408889634


def _pack(x):
    return pltpu.bitcast(x.astype(BF16), U32)


def _unpack(x):
    return pltpu.bitcast(x, BF16)


def _ln(x):
    m = jnp.mean(x, axis=-1, keepdims=True)
    xc = x - m
    v = jnp.mean(xc * xc, axis=-1, keepdims=True)
    return xc * lax.rsqrt(v + EPS)


def _dot(a, b):
    return jnp.dot(a, b, preferred_element_type=F32)


def _make(NG=8, D=4, NS=4, XH=8):
    HG = H // NG
    GW = HG * DH
    CH = 128
    NCH = DM // CH
    WOC = 4

    def kernel(x_hbm, mem0_ref, wq_hbm, wk_hbm, wv_hbm, wo_hbm, wg_hbm, wu_hbm, wd_hbm,
               y_hbm,
               wqkv_s, wo_s, wg_s, wu_s, wd_s, st3_s, wo_st, wg_st, wu_st, wd_st,
               x0_s, htok_s, acc_s, x1_s, x2_s, fres_s, y_s, sem3, semw, osem):
        srcs = [wq_hbm, wk_hbm, wv_hbm]
        jobs = [(m, i) for m in range(3) for i in range(NCH)]

        def cp3(j):
            m, i = jobs[j]
            return pltpu.make_async_copy(srcs[m].at[pl.ds(i * CH, CH)], st3_s.at[j % NS], sem3.at[j % NS])
        XR = XH * SEG
        cp_xh = pltpu.make_async_copy(x_hbm.at[pl.ds(0, XR)], x0_s.at[pl.ds(0, XR)], semw.at[0])
        cp_xr = pltpu.make_async_copy(x_hbm.at[pl.ds(XR, S - XR)], x0_s.at[pl.ds(XR, S - XR)], semw.at[1])
        WOR = H * DH // WOC
        cp_wo = [pltpu.make_async_copy(wo_hbm.at[pl.ds(c * WOR, WOR)], wo_st.at[pl.ds(c * WOR, WOR)], semw.at[2 + c])
                 for c in range(WOC)]
        cp_wg = pltpu.make_async_copy(wg_hbm, wg_st, semw.at[2 + WOC])
        cp_wu = pltpu.make_async_copy(wu_hbm, wu_st, semw.at[3 + WOC])
        cp_wd = pltpu.make_async_copy(wd_hbm, wd_st, semw.at[4 + WOC])

        def convert2(src, dst, r0, nrows):
            def body(b, c):
                dst[pl.ds(pl.multiple_of(r0 // 2 + b * 8, 8), 8), :] = pltpu.bitcast(
                    src[pl.ds(pl.multiple_of(r0 + b * 16, 16), 16), :], U32)
                return c
            lax.fori_loop(0, nrows // 16, body, 0)

        cp_xh.start()
        for j in range(NS):
            cp3(j).start()
        for j, (m, i) in enumerate(jobs):
            cp3(j).wait()

            def body(b, c, m=m, i=i, slot=j % NS):
                d0 = pl.multiple_of(b * 16, 16)
                s32 = pltpu.bitcast(st3_s[slot, pl.ds(d0, 16)], U32).reshape(8, 2, 16, DH)
                a = jnp.swapaxes(s32[:, 0], 0, 1)
                bb = jnp.swapaxes(s32[:, 1], 0, 1)
                lo = (a & U32(0xFFFF)) | (bb << 16)
                hi = (a >> 16) | (bb & U32(0xFFFF0000))
                r0 = pl.multiple_of(i * (CH // 2) + b * 8, 8)
                for hp in range(16):
                    for par, val in ((0, lo), (1, hi)):
                        hh = 2 * hp + par
                        g, hg = hh // HG, hh % HG
                        wqkv_s[g, pl.ds(r0, 8), pl.ds(m * GW + hg * DH, DH)] = val[hp]
                return c
            lax.fori_loop(0, CH // 16, body, 0)
            if j + NS < len(jobs):
                cp3(j + NS).start()
            elif j + NS == len(jobs):
                for c in cp_wo:
                    c.start()
                cp_wg.start()
                cp_wu.start()
                cp_wd.start()
                cp_xr.start()
        cp_xh.wait()

        c1 = (DH ** -0.5) * LOG2E

        def make_mask(rows, tok_layers):
            row = lax.broadcasted_iota(jnp.int32, (rows, rows), 0)
            col = lax.broadcasted_iota(jnp.int32, (rows, rows), 1)

            def layer(i):
                lay = jnp.where(i < M, 0, 1)
                for b, l in enumerate(tok_layers):
                    lay = jnp.where(i >= MP + b * SEG, l, lay)
                return lay
            return (layer(row) == layer(col)) & ((row < MP) | (col < MP) | (row >= col))

        def qkv(hh, g):
            r = _dot(hh, _unpack(wqkv_s[g]))
            q = [r[:, j * DH:(j + 1) * DH].astype(BF16) for j in range(HG)]
            k = [r[:, GW + j * DH:GW + (j + 1) * DH].astype(BF16) for j in range(HG)]
            v = [r[:, 2 * GW + j * DH:2 * GW + (j + 1) * DH].astype(BF16) for j in range(HG)]
            return q, k, v

        def scores(q, k):
            return [lax.dot_general(q[j], k[j], (((1,), (1,)), ((), ())), preferred_element_type=F32)
                    for j in range(HG)]

        def softmax_pv(ss, v, mask):
            os_ = []
            for j in range(HG):
                s = jnp.where(mask, ss[j], NEG)
                mx = jnp.max(s, axis=-1, keepdims=True)
                e = jnp.exp2((s - mx) * c1)
                l = jnp.sum(e, axis=-1, keepdims=True)
                p = (e * pl.reciprocal(l, approx=True)).astype(BF16)
                os_.append(_dot(p, v[j]))
            return jnp.concatenate(os_, axis=1).astype(BF16)

        def wo(o, g, acc):
            r = _dot(o, _unpack(wo_s[pl.ds(g * (GW // 2), GW // 2), :]))
            return r if acc is None else acc + r

        def ffn_a(f, c0, c1_):
            gg = _dot(f, _unpack(wg_s[:, c0:c1_]))
            uu = _dot(f, _unpack(wu_s[:, c0:c1_]))
            return (uu * (0.5 * jnp.tanh(0.5 * gg) + 0.5)).astype(BF16)

        def ffn_b(a):
            return _dot(a, _unpack(wd_s[...]))

        def ffn32(r):
            return r + ffn_b(ffn_a(_ln(r).astype(BF16), 0, FF))

        def attention(hh, mask, fillers, mid=None):
            qs, ss, oo = {}, {}, {}
            acc = None
            late = mid is not None
            for i in range(NG + 3):
                if i < NG:
                    qs[i] = qkv(hh, i)
                elif i - NG < len(fillers):
                    fillers[i - NG]()
                if 0 <= i - 3 < NG and not late:
                    acc = wo(oo.pop(i - 3), i - 3, acc)
                if 0 <= i - 2 < NG:
                    oo[i - 2] = softmax_pv(ss.pop(i - 2), qs.pop(i - 2)[2], mask)
                if 0 <= i - 1 < NG:
                    ss[i - 1] = scores(qs[i - 1][0], qs[i - 1][1])
            if late:
                o_all = jnp.concatenate([oo[g] for g in range(NG)], axis=1)
                o_all = mid(o_all)
                acc = _dot(o_all, _unpack(wo_s[...]))
            return acc

        def out_copy(seg, slot):
            return pltpu.make_async_copy(y_s.at[slot], y_hbm.at[pl.ds(seg * SEG, SEG)], osem.at[slot])

        def x0seg(i):
            i = jnp.clip(i, 0, NSEG - 1)
            return x0_s[pl.ds(pl.multiple_of(i * SEG, SEG), SEG), :].astype(F32)

        def emit_y(yseg, yv):
            yslot = yseg % 2

            @pl.when(yseg >= 2)
            def _():
                out_copy(yseg - 2, yslot).wait()
            y_s[yslot] = yv.astype(BF16)

            @pl.when(yseg >= 0)
            def _():
                out_copy(yseg, yslot).start()

        def mem_pair(t, l1_live=True):
            mem0 = mem0_ref[...].astype(F32)
            mem1 = acc_s[:M, :] if l1_live else jnp.zeros((M, DM), F32)
            mem2 = jnp.where(t <= D, mem0, acc_s[M:MP, :])
            return jnp.concatenate([mem1, mem2], axis=0).astype(BF16)

        mem0 = mem0_ref[...].astype(F32)
        htok_s[0] = _pack(_ln(x0seg(0)))
        htok_s[1] = jnp.zeros((SEG // 2, DM), U32)
        acc_s[...] = jnp.concatenate([mem0, mem0, jnp.zeros((2 * SEG, DM), F32)], axis=0)
        x2_s[...] = jnp.zeros(x2_s.shape, F32)

        mask1 = make_mask(MP + SEG, [0])

        def pro(t, carry):
            x1_s[(t + D - 1) % D] = x0seg(t - 1) + acc_s[MP:MP + SEG, :]
            hh = jnp.concatenate([mem_pair(t), _unpack(htok_s[0])], axis=0)
            tok1 = _ln(x0seg(t + 1))

            def mid(o_all):
                o_s = o_all

                @pl.when(t == 0)
                def _():
                    for c in range(WOC):
                        cp_wo[c].wait()
                        convert2(wo_st, wo_s, c * WOR, WOR)
                return o_s
            acc = attention(hh, mask1, [], mid=mid)
            acc_s[:MP + SEG, :] = acc
            htok_s[0] = _pack(tok1)

            @pl.when(t == D - 3)
            def _():
                cp_wg.wait()
                convert2(wg_st, wg_s, 0, DM)

            @pl.when(t == D - 2)
            def _():
                cp_wu.wait()
                convert2(wu_st, wu_s, 0, DM)

            @pl.when(t == D - 1)
            def _():
                cp_wd.wait()
                convert2(wd_st, wd_s, 0, FF)
                cp_xr.wait()
            return carry
        lax.fori_loop(0, D, pro, 0)
        x2 = ffn32(x1_s[0])
        x2_s[(D - 1) % 2] = x2
        htok_s[1] = _pack(_ln(x2))

        mask2 = make_mask(MP + 2 * SEG, [0, 1])

        def step(t, carry):
            x1_s[(t - 1) % D] = x0seg(t - 1) + acc_s[MP:MP + SEG, :]
            hh = jnp.concatenate([mem_pair(t), _unpack(htok_s[0]), _unpack(htok_s[1])], axis=0)
            slot = t % 2
            res = jnp.concatenate([x1_s[(t - D + 1) % D], x2_s[slot] + acc_s[MP + SEG:, :]], axis=0)
            fin = _ln(res).astype(BF16)
            tok1 = _ln(x0seg(t + 1))
            acts = []
            fo = []
            fillers = [lambda: acts.append(ffn_a(fin, 0, FF // 2)),
                       lambda: acts.append(ffn_a(fin, FF // 2, FF)),
                       lambda: fo.append(ffn_b(jnp.concatenate(acts, axis=1)))]
            acc = attention(hh, mask2, fillers)
            xo = res + fo[0]
            x2_new = xo[:SEG]
            acc_s[...] = acc
            x2_s[slot] = x2_new
            htok_s[0] = _pack(tok1)
            htok_s[1] = _pack(_ln(x2_new))
            emit_y(t - D - 1, xo[SEG:])
            return carry
        lax.fori_loop(D, NSEG, step, 0)

        mask3 = make_mask(MP + SEG, [1])

        def epi(t, carry):
            slot = t % 2

            @pl.when(t == NSEG)
            def _():
                x1_s[(t - 1) % D] = x0seg(t - 1) + acc_s[MP:MP + SEG, :]
            fres_s[0] = x1_s[(t - D + 1) % D]
            fres_s[1] = x2_s[slot] + acc_s[MP + SEG:, :]

            @pl.when(t < NSEG + D)
            def _():
                hh = jnp.concatenate([mem_pair(t, l1_live=False), _unpack(htok_s[1])], axis=0)
                acc = attention(hh, mask3, [])
                acc_s[:MP, :] = acc[:MP]
                acc_s[MP + SEG:, :] = acc[MP:]

            def f(w, c):
                xo = ffn32(fres_s[w])

                @pl.when(w == 0)
                def _():
                    x2_s[slot] = xo
                    htok_s[1] = _pack(_ln(xo))

                @pl.when(w == 1)
                def _():
                    emit_y(t - D - 1, xo)
                return c
            lax.fori_loop(jnp.where(t < NSEG + D - 1, 0, 1), 2, f, 0)
            return carry
        lax.fori_loop(NSEG, NSEG + D + 1, epi, 0)
        out_copy(NSEG - 2, 0).wait()
        out_copy(NSEG - 1, 1).wait()

    def run(A_x, A_mem0, A_Wq, A_Wk, A_Wv, A_Wo, A_seg_len, B_x, B_w_gate, B_w_up, B_w_down):
        any_spec = pl.BlockSpec(memory_space=pl.ANY)
        out = pl.pallas_call(
            kernel,
            out_shape=jax.ShapeDtypeStruct((S, DM), BF16),
            in_specs=[any_spec, pl.BlockSpec(memory_space=pltpu.VMEM)] + [any_spec] * 7,
            out_specs=any_spec,
            scratch_shapes=[
                pltpu.VMEM((NG, DM // 2, 3 * GW), U32),
                pltpu.VMEM((H * DH // 2, DM), U32),
                pltpu.VMEM((DM // 2, FF), U32),
                pltpu.VMEM((DM // 2, FF), U32),
                pltpu.VMEM((FF // 2, DM), U32),
                pltpu.VMEM((NS, CH, H, DH), BF16),
                pltpu.VMEM((H * DH, DM), BF16),
                pltpu.VMEM((DM, FF), BF16),
                pltpu.VMEM((DM, FF), BF16),
                pltpu.VMEM((FF, DM), BF16),
                pltpu.VMEM((S, DM), BF16),
                pltpu.VMEM((2, SEG // 2, DM), U32),
                pltpu.VMEM((MP + 2 * SEG, DM), F32),
                pltpu.VMEM((D, SEG, DM), F32),
                pltpu.VMEM((2, SEG, DM), F32),
                pltpu.VMEM((2, SEG, DM), F32),
                pltpu.VMEM((2, SEG, DM), BF16),
                pltpu.SemaphoreType.DMA((NS,)),
                pltpu.SemaphoreType.DMA((5 + WOC,)),
                pltpu.SemaphoreType.DMA((2,)),
            ],
            compiler_params=pltpu.CompilerParams(vmem_limit_bytes=120 * 1024 * 1024),
            name="memtr",
        )(A_x.reshape(S, DM), A_mem0.reshape(M, DM), A_Wq, A_Wk, A_Wv, A_Wo.reshape(H * DH, DM),
          B_w_gate, B_w_up, B_w_down)
        return out.reshape(1, S, DM)
    return run


_run = _make()


@functools.partial(jax.jit, static_argnames=("A_seg_len",))
def pallas_interleave_layers__memory_aug_recurrent_mem_tr__glu_gated_glu__prompt_kernel(
    A_x, A_mem0, A_Wq, A_Wk, A_Wv, A_Wo, A_seg_len, B_x, B_w_gate, B_w_up, B_w_down,
):
    assert A_seg_len == SEG
    assert A_x.shape == (1, S, DM) and A_mem0.shape == (1, M, DM)
    assert A_Wq.shape == (DM, H, DH) and A_Wo.shape == (H, DH, DM)
    assert B_w_gate.shape == (DM, FF) and B_w_down.shape == (FF, DM)
    return _run(A_x, A_mem0, A_Wq, A_Wk, A_Wv, A_Wo, A_seg_len, B_x, B_w_gate, B_w_up, B_w_down)
```

```python
import functools
import jax
import jax.numpy as jnp
from jax import lax
from jax.experimental import pallas as pl
from jax.experimental.pallas import tpu as pltpu

S, DM, H, DH, M, SEG, FF = 2048, 1024, 32, 128, 8, 32, 3584
NSEG = S // SEG
MP = 2 * M
U32 = jnp.uint32
BF16 = jnp.bfloat16
F32 = jnp.float32
EPS = 1e-5
NEG = -1e9
LOG2E = 1.4426950408889634


def _pack(x):
    return pltpu.bitcast(x.astype(BF16), U32)


def _unpack(x):
    return pltpu.bitcast(x, BF16)


def _ln(x):
    m = jnp.mean(x, axis=-1, keepdims=True)
    xc = x - m
    v = jnp.mean(xc * xc, axis=-1, keepdims=True)
    return xc * lax.rsqrt(v + EPS)


def _dot(a, b):
    return jnp.dot(a, b, preferred_element_type=F32)


def _make(D=3, NP=9):
    NG = 8
    HG = H // NG
    GW = HG * DH
    NOCT = H // 8
    WOC = 4
    R = NP + D
    XH = NP + D + 1

    def kernel(x_hbm, mem0_ref, wq_hbm, wk_hbm, wv_hbm, wo_hbm, wg_hbm, wu_hbm, wd_hbm,
               y_hbm,
               wq_s, wk_s, wv_s, wo_s, wg_s, wu_s, wd_s, st3_s, wo_st, wg_st, wu_st, wd_st,
               x0_s, ptok_s, ring_s, htok_s, acc_s, x1_s, x2_s, fres_s, y_s, sem3, semw, osem):
        srcs = [wq_hbm, wk_hbm, wv_hbm]
        w3_s = [wq_s, wk_s, wv_s]

        def cp3(o, m):
            return pltpu.make_async_copy(srcs[m].at[:, pl.ds(pl.multiple_of(o * 8, 8), 8), :],
                                         st3_s.at[o % 2, m], sem3.at[o % 2, m])
        XR = XH * SEG
        cp_xh = pltpu.make_async_copy(x_hbm.at[pl.ds(0, XR)], x0_s.at[pl.ds(0, XR)], semw.at[0])
        cp_xr = pltpu.make_async_copy(x_hbm.at[pl.ds(XR, S - XR)], x0_s.at[pl.ds(XR, S - XR)], semw.at[1])
        WOR = H * DH // WOC
        cp_wo = [pltpu.make_async_copy(wo_hbm.at[pl.ds(c * WOR, WOR)], wo_st.at[pl.ds(c * WOR, WOR)], semw.at[2 + c])
                 for c in range(WOC)]
        cp_wg = pltpu.make_async_copy(wg_hbm, wg_st, semw.at[2 + WOC])
        cp_wu = pltpu.make_async_copy(wu_hbm, wu_st, semw.at[3 + WOC])
        cp_wd = pltpu.make_async_copy(wd_hbm, wd_st, semw.at[4 + WOC])

        def issue(descs):
            def body(i, c):
                for k, d in enumerate(descs):
                    pl.when(i == k)(d.start)
                return c
            lax.fori_loop(0, len(descs), body, 0)

        def x0seg(i):
            i = jnp.clip(i, 0, NSEG - 1)
            return x0_s[pl.ds(pl.multiple_of(i * SEG, SEG), SEG), :].astype(F32)

        sub8 = lax.broadcasted_iota(jnp.int32, (8, DH), 0)

        def conv3(o, m, b0=0, b1=DM // 16):
            for b in range(b0, b1):
                s32 = pltpu.bitcast(st3_s[o % 2, m, pl.ds(b * 16, 16)], U32).reshape(8, 2, 4, DH)
                sides = []
                for par in range(2):
                    P = [jnp.concatenate([s32[k, par], s32[k + 4, par]], axis=0) for k in range(4)]
                    for dist in (1, 2):
                        msk = (sub8 & dist) == 0
                        Q = list(P)
                        for k in range(4):
                            if k & dist == 0:
                                Q[k] = jnp.where(msk, P[k], pltpu.roll(P[k + dist], dist, 0))
                                Q[k + dist] = jnp.where(msk, pltpu.roll(P[k], 8 - dist, 0), P[k + dist])
                        P = Q
                    sides.append(P)
                lo = [(sides[0][hp] & U32(0xFFFF)) | (sides[1][hp] << 16) for hp in range(4)]
                hi = [(sides[0][hp] >> 16) | (sides[1][hp] & U32(0xFFFF0000)) for hp in range(4)]
                for hp in range(4):
                    for par, val in ((0, lo), (1, hi)):
                        hh = 2 * hp + par
                        w3_s[m][2 * o + hh // HG, pl.ds(b * 8, 8), pl.ds((hh % HG) * DH, DH)] = val[hp]

        def pmm(o, m):
            for pc in range(8):
                pmm_piece(o, m, pc)

        def pmm_piece(o, m, pc):
            p = _unpack(ptok_s[...])
            g = 2 * o + pc // 4
            cs = pl.ds((pc % 4) * DH, DH)
            r = _pack(_dot(p, _unpack(w3_s[m][g, :, cs])))
            for sg in range(NP):
                ring_s[sg, g, m, :, cs] = r[sg * 16:(sg + 1) * 16]

        with jax.named_scope('P'):
            issue([cp3(0, 0), cp_xh] + [cp3(o, m) for o in range(2) for m in range(3) if o + m > 0])

            def pstage(o, carry):
                for m in range(3):
                    if m == 0:
                        @pl.when(o > 0)
                        def _():
                            pmm(o - 1, 2)

                        @pl.when(o + 2 == NOCT)
                        def _():
                            issue(cp_wo + [cp_wg, cp_wu, cp_wd, cp_xr])
                        cp3(o, 0).wait()
                    else:
                        if m == 1:
                            @pl.when(o == 0)
                            def _():
                                cp_xh.wait()
                                for sg in range(NP):
                                    ptok_s[pl.ds(sg * 16, 16), :] = _pack(_ln(x0seg(sg)))
                        pmm(o, m - 1)
                        cp3(o, m).wait()
                    conv3(o, m)

                    @pl.when(o + 2 < NOCT)
                    def _():
                        cp3(o + 2, m).start()
                return carry
            lax.fori_loop(0, NOCT, pstage, 0)
            pmm(NOCT - 1, 2)

        c1 = (DH ** -0.5) * LOG2E

        def make_mask(rows, tok_layers):
            row = lax.broadcasted_iota(jnp.int32, (rows, rows), 0)
            col = lax.broadcasted_iota(jnp.int32, (rows, rows), 1)

            def layer(i):
                lay = jnp.where(i < M, 0, 1)
                for b, l in enumerate(tok_layers):
                    lay = jnp.where(i >= MP + b * SEG, l, lay)
                return lay
            return (layer(row) == layer(col)) & ((row < MP) | (col < MP) | (row >= col))

        def split(r):
            return [r[:, j * DH:(j + 1) * DH] for j in range(HG)]

        def qkv_plain(hh):
            def get(g):
                return [[x.astype(BF16) for x in split(_dot(hh, _unpack(w3_s[m][g])))] for m in range(3)]
            return get

        def qkv_ring(hh, rd, wr):
            def get(g):
                out = []
                for m in range(3):
                    r = _dot(hh, _unpack(w3_s[m][g]))
                    old = split(_unpack(ring_s[rd, g, m]))
                    rs = split(r)
                    if wr is None:
                        out.append([jnp.concatenate([rs[j][:MP].astype(BF16), old[j], rs[j][MP:].astype(BF16)], axis=0)
                                    for j in range(HG)])
                    else:
                        ring_s[wr, g, m] = _pack(r[MP:])
                        out.append([jnp.concatenate([rs[j][:MP].astype(BF16), old[j]], axis=0) for j in range(HG)])
                return out
            return get

        def scores(q, k):
            return [lax.dot_general(q[j], k[j], (((1,), (1,)), ((), ())), preferred_element_type=F32)
                    for j in range(HG)]

        def softmax_pv(ss, v, mask):
            os_ = []
            for j in range(HG):
                s = jnp.where(mask, ss[j], NEG)
                mx = jnp.max(s, axis=-1, keepdims=True)
                e = jnp.exp2((s - mx) * c1)
                l = jnp.sum(e, axis=-1, keepdims=True)
                p = (e * pl.reciprocal(l, approx=True)).astype(BF16)
                os_.append(_dot(p, v[j]))
            return jnp.concatenate(os_, axis=1).astype(BF16)

        def wo(o, g, acc):
            r = _dot(o, _unpack(wo_s[pl.ds(g * (GW // 2), GW // 2), :]))
            return r if acc is None else acc + r

        def ffn_a(f, c0, c1_):
            gg = _dot(f, _unpack(wg_s[:, c0:c1_]))
            uu = _dot(f, _unpack(wu_s[:, c0:c1_]))
            return (uu * (0.5 * jnp.tanh(0.5 * gg) + 0.5)).astype(BF16)

        def ffn_b(a):
            return _dot(a, _unpack(wd_s[...]))

        def ffn32(r):
            return r + ffn_b(ffn_a(_ln(r).astype(BF16), 0, FF))

        def attention(get, mask, fillers, late_wo=None):
            qs, ss, oo = {}, {}, {}
            acc = None
            for i in range(NG + 3):
                if i < NG:
                    qs[i] = get(i)
                elif i - NG < len(fillers):
                    fillers[i - NG]()
                if 0 <= i - 3 < NG and late_wo is None:
                    acc = wo(oo.pop(i - 3), i - 3, acc)
                if 0 <= i - 2 < NG:
                    oo[i - 2] = softmax_pv(ss.pop(i - 2), qs.pop(i - 2)[2], mask)
                if 0 <= i - 1 < NG:
                    ss[i - 1] = scores(qs[i - 1][0], qs[i - 1][1])
            if late_wo is not None:
                acc = late_wo(oo)
            return acc

        def out_copy(seg, slot):
            return pltpu.make_async_copy(y_s.at[slot], y_hbm.at[pl.ds(seg * SEG, SEG)], osem.at[slot])

        def emit_y(yseg, yv):
            yslot = yseg % 2

            @pl.when(yseg >= 2)
            def _():
                out_copy(yseg - 2, yslot).wait()
            y_s[yslot] = yv.astype(BF16)

            @pl.when(yseg >= 0)
            def _():
                out_copy(yseg, yslot).start()

        def mem_pair(t, l1_live=True):
            mem0 = mem0_ref[...].astype(F32)
            mem1 = acc_s[:M, :] if l1_live else jnp.zeros((M, DM), F32)
            mem2 = jnp.where(t <= D, mem0, acc_s[M:MP, :])
            return jnp.concatenate([mem1, mem2], axis=0).astype(BF16)

        def conv_all(src, dst):
            dst[...] = pltpu.bitcast(src[...], U32)

        mem0 = mem0_ref[...].astype(F32)
        acc_s[...] = jnp.concatenate([mem0, mem0, jnp.zeros((2 * SEG, DM), F32)], axis=0)
        x2_s[...] = jnp.zeros(x2_s.shape, F32)

        mask1 = make_mask(MP + SEG, [0])

        def pro(t, first):
            if not first:
                x1_s[(t - 1) % D] = x0seg(t - 1) + acc_s[MP:MP + SEG, :]
            hm = jnp.concatenate([acc_s[:M, :], mem0_ref[...].astype(F32)], axis=0).astype(BF16)
            hh = jnp.concatenate([hm, _ln(x0seg(t + NP)).astype(BF16)], axis=0)
            late = None
            if first:
                def late(oo):
                    acc = None
                    gpc = NG // WOC
                    for c in range(WOC):
                        cp_wo[c].wait()
                        for g in range(c * gpc, (c + 1) * gpc):
                            wov = pltpu.bitcast(wo_st[pl.ds(g * GW, GW), :], U32)
                            wo_s[pl.ds(g * (GW // 2), GW // 2), :] = wov
                            r = _dot(oo[g], _unpack(wov))
                            acc = r if acc is None else acc + r
                    return acc
            acc = attention(qkv_ring(hh, t, t + NP), mask1, [], late_wo=late)
            acc_s[:MP + SEG, :] = acc

        with jax.named_scope('PRO0'):
            pro(0, True)

        def pro_rest(t, carry):
            pro(t, False)
            return carry
        with jax.named_scope('PRO1'):
            lax.fori_loop(1, D, pro_rest, 0)
        with jax.named_scope('FFN0'):
            cp_wg.wait()
            cp_wu.wait()
            cp_wd.wait()
            r0 = x1_s[0]
            f0 = _ln(r0).astype(BF16)
            acts0 = []
            FC = 512
            for c0 in range(0, FF, FC):
                wgv = pltpu.bitcast(wg_st[:, c0:c0 + FC], U32)
                wuv = pltpu.bitcast(wu_st[:, c0:c0 + FC], U32)
                wg_s[:, c0:c0 + FC] = wgv
                wu_s[:, c0:c0 + FC] = wuv
                gg = _dot(f0, _unpack(wgv))
                uu = _dot(f0, _unpack(wuv))
                acts0.append((uu * (0.5 * jnp.tanh(0.5 * gg) + 0.5)).astype(BF16))
            x2 = r0
            for i, c0 in enumerate(range(0, FF, FC)):
                wdv = pltpu.bitcast(wd_st[c0:c0 + FC, :], U32)
                wd_s[c0 // 2:(c0 + FC) // 2, :] = wdv
                x2 = x2 + _dot(acts0[i], _unpack(wdv))
            x2_s[(D - 1) % 2] = x2
            htok_s[1] = _pack(_ln(x2))
            cp_xr.wait()

        mask2 = make_mask(MP + 2 * SEG, [0, 1])

        def step(t, carry, ringed):
            x1_s[(t - 1) % D] = x0seg(t - 1) + acc_s[MP:MP + SEG, :]
            if ringed:
                get = qkv_ring(jnp.concatenate([mem_pair(t), _unpack(htok_s[1])], axis=0), t, None)
            else:
                get = qkv_plain(jnp.concatenate([mem_pair(t), _unpack(htok_s[0]), _unpack(htok_s[1])], axis=0))
            slot = t % 2
            res = jnp.concatenate([x1_s[(t - D + 1) % D], x2_s[slot] + acc_s[MP + SEG:, :]], axis=0)
            fin = _ln(res).astype(BF16)
            tok1 = _ln(x0seg(t + 1))
            acts = []
            fo = []
            fillers = [lambda: acts.append(ffn_a(fin, 0, FF // 2)),
                       lambda: acts.append(ffn_a(fin, FF // 2, FF)),
                       lambda: fo.append(ffn_b(jnp.concatenate(acts, axis=1)))]
            acc = attention(get, mask2, fillers)
            xo = res + fo[0]
            x2_new = xo[:SEG]
            acc_s[...] = acc
            x2_s[slot] = x2_new
            htok_s[0] = _pack(tok1)
            htok_s[1] = _pack(_ln(x2_new))
            emit_y(t - D - 1, xo[SEG:])
            return carry
        with jax.named_scope('PDUAL'):
            lax.fori_loop(D, D + NP, functools.partial(step, ringed=True), 0)
        with jax.named_scope('MAIN'):
            lax.fori_loop(D + NP, NSEG, functools.partial(step, ringed=False), 0)

        mask3 = make_mask(MP + SEG, [1])

        def epi(t, carry):
            slot = t % 2

            @pl.when(t == NSEG)
            def _():
                x1_s[(t - 1) % D] = x0seg(t - 1) + acc_s[MP:MP + SEG, :]
            fres_s[0] = x1_s[(t - D + 1) % D]
            fres_s[1] = x2_s[slot] + acc_s[MP + SEG:, :]

            @pl.when(t < NSEG + D)
            def _():
                hh = jnp.concatenate([mem_pair(t, l1_live=False), _unpack(htok_s[1])], axis=0)
                acc = attention(qkv_plain(hh), mask3, [])
                acc_s[:MP, :] = acc[:MP]
                acc_s[MP + SEG:, :] = acc[MP:]

            def f(w, c):
                xo = ffn32(fres_s[w])

                @pl.when(w == 0)
                def _():
                    x2_s[slot] = xo
                    htok_s[1] = _pack(_ln(xo))

                @pl.when(w == 1)
                def _():
                    emit_y(t - D - 1, xo)
                return c
            lax.fori_loop(jnp.where(t < NSEG + D - 1, 0, 1), 2, f, 0)
            return carry
        with jax.named_scope('EPI'):
            lax.fori_loop(NSEG, NSEG + D + 1, epi, 0)
        out_copy(NSEG - 2, 0).wait()
        out_copy(NSEG - 1, 1).wait()

    def run(A_x, A_mem0, A_Wq, A_Wk, A_Wv, A_Wo, A_seg_len, B_x, B_w_gate, B_w_up, B_w_down):
        any_spec = pl.BlockSpec(memory_space=pl.ANY)
        out = pl.pallas_call(
            kernel,
            out_shape=jax.ShapeDtypeStruct((S, DM), BF16),
            in_specs=[any_spec, pl.BlockSpec(memory_space=pltpu.VMEM)] + [any_spec] * 7,
            out_specs=any_spec,
            scratch_shapes=[
                pltpu.VMEM((NG, DM // 2, GW), U32),
                pltpu.VMEM((NG, DM // 2, GW), U32),
                pltpu.VMEM((NG, DM // 2, GW), U32),
                pltpu.VMEM((H * DH // 2, DM), U32),
                pltpu.VMEM((DM // 2, FF), U32),
                pltpu.VMEM((DM // 2, FF), U32),
                pltpu.VMEM((FF // 2, DM), U32),
                pltpu.VMEM((2, 3, DM, 8, DH), BF16),
                pltpu.VMEM((H * DH, DM), BF16),
                pltpu.VMEM((DM, FF), BF16),
                pltpu.VMEM((DM, FF), BF16),
                pltpu.VMEM((FF, DM), BF16),
                pltpu.VMEM((S, DM), BF16),
                pltpu.VMEM((NP * SEG // 2, DM), U32),
                pltpu.VMEM((R, NG, 3, SEG // 2, GW), U32),
                pltpu.VMEM((2, SEG // 2, DM), U32),
                pltpu.VMEM((MP + 2 * SEG, DM), F32),
                pltpu.VMEM((D, SEG, DM), F32),
                pltpu.VMEM((2, SEG, DM), F32),
                pltpu.VMEM((2, SEG, DM), F32),
                pltpu.VMEM((2, SEG, DM), BF16),
                pltpu.SemaphoreType.DMA((2, 3)),
                pltpu.SemaphoreType.DMA((5 + WOC,)),
                pltpu.SemaphoreType.DMA((2,)),
            ],
            compiler_params=pltpu.CompilerParams(vmem_limit_bytes=124 * 1024 * 1024),
            name="memtr",
        )(A_x.reshape(S, DM), A_mem0.reshape(M, DM), A_Wq, A_Wk, A_Wv, A_Wo.reshape(H * DH, DM),
          B_w_gate, B_w_up, B_w_down)
        return out.reshape(1, S, DM)
    return run


_run = _make()


@functools.partial(jax.jit, static_argnames=("A_seg_len",))
def pallas_interleave_layers__memory_aug_recurrent_mem_tr__glu_gated_glu__prompt_kernel(
    A_x, A_mem0, A_Wq, A_Wk, A_Wv, A_Wo, A_seg_len, B_x, B_w_gate, B_w_up, B_w_down,
):
    assert A_seg_len == SEG
    assert A_x.shape == (1, S, DM) and A_mem0.shape == (1, M, DM)
    assert A_Wq.shape == (DM, H, DH) and A_Wo.shape == (H, DH, DM)
    assert B_w_gate.shape == (DM, FF) and B_w_down.shape == (FF, DM)
    return _run(A_x, A_mem0, A_Wq, A_Wk, A_Wv, A_Wo, A_seg_len, B_x, B_w_gate, B_w_up, B_w_down)
```

```python
import functools
import jax
import jax.numpy as jnp
from jax import lax
from jax.experimental import pallas as pl
from jax.experimental.pallas import tpu as pltpu

S, DM, H, DH, M, SEG, FF = 2048, 1024, 32, 128, 8, 32, 3584
NSEG = S // SEG
MP = 2 * M
U32 = jnp.uint32
BF16 = jnp.bfloat16
F32 = jnp.float32
EPS = 1e-5
NEG = -1e9
LOG2E = 1.4426950408889634


def _pack(x):
    return pltpu.bitcast(x.astype(BF16), U32)


def _unpack(x):
    return pltpu.bitcast(x, BF16)


def _ln(x):
    m = jnp.mean(x, axis=-1, keepdims=True)
    xc = x - m
    v = jnp.mean(xc * xc, axis=-1, keepdims=True)
    return xc * lax.rsqrt(v + EPS)


def _dot(a, b):
    return jnp.dot(a, b, preferred_element_type=F32)


def _make(D=3, NP=11, NOBC=0):
    NG = 8
    HG = H // NG
    GW = HG * DH
    NOCT = H // 8
    WOC = 4
    R = NP + D
    XR2 = 4
    assert D == 3
    XH = NP + D + 1

    def kernel(x_hbm, mem0_hbm, wq_hbm, wk_hbm, wv_hbm, wo_hbm, wg_hbm, wu_hbm, wd_hbm,
               y_hbm,
               wq_s, wk_s, wv_s, wo_s, wg_s, wu_s, wd_s, st3_s, wo_st, wg_st, wu_st, wd_st,
               x0_s, mem0_ref, ptok_s, ring_s, htok_s, acc_s, x1_s, x2_s, fres_s, y_s, sem3, semw, osem):
        srcs = [wq_hbm, wk_hbm, wv_hbm]
        w3_s = [wq_s, wk_s, wv_s]

        def cp3(o, m):
            return pltpu.make_async_copy(srcs[m].at[:, pl.ds(pl.multiple_of(o * 8, 8), 8), :],
                                         st3_s.at[o % 2, m], sem3.at[o % 2, m])
        XR = XH * SEG
        cp_xh = pltpu.make_async_copy(x_hbm.at[pl.ds(0, XR)], x0_s.at[pl.ds(0, XR)], semw.at[0])
        cp_xr = pltpu.make_async_copy(x_hbm.at[pl.ds(XR, S - XR)], x0_s.at[pl.ds(XR, S - XR)], semw.at[1])
        cp_m0 = pltpu.make_async_copy(mem0_hbm, mem0_ref, semw.at[5 + WOC])
        WOR = H * DH // WOC
        cp_wo = [pltpu.make_async_copy(wo_hbm.at[pl.ds(c * WOR, WOR)], wo_st.at[pl.ds(c * WOR, WOR)], semw.at[2 + c])
                 for c in range(WOC)]
        cp_wg = pltpu.make_async_copy(wg_hbm, wg_st, semw.at[2 + WOC])
        cp_wu = pltpu.make_async_copy(wu_hbm, wu_st, semw.at[3 + WOC])
        cp_wd = pltpu.make_async_copy(wd_hbm, wd_st, semw.at[4 + WOC])

        def issue(descs):
            def body(i, c):
                for k, d in enumerate(descs):
                    pl.when(i == k)(d.start)
                return c
            lax.fori_loop(0, len(descs), body, 0)

        def x0seg(i):
            i = jnp.clip(i, 0, NSEG - 1)
            return x0_s[pl.ds(pl.multiple_of(i * SEG, SEG), SEG), :].astype(F32)

        sub8 = lax.broadcasted_iota(jnp.int32, (8, DH), 0)

        def conv_block(o, m, b):
            s32 = pltpu.bitcast(st3_s[o % 2, m, pl.ds(b * 16, 16)], U32).reshape(8, 2, 4, DH)
            sides = []
            for par in range(2):
                P = [jnp.concatenate([s32[k, par], s32[k + 4, par]], axis=0) for k in range(4)]
                for dist in (1, 2):
                    msk = (sub8 & dist) == 0
                    Q = list(P)
                    for k in range(4):
                        if k & dist == 0:
                            Q[k] = jnp.where(msk, P[k], pltpu.roll(P[k + dist], dist, 0))
                            Q[k + dist] = jnp.where(msk, pltpu.roll(P[k], 8 - dist, 0), P[k + dist])
                    P = Q
                sides.append(P)
            out = []
            for hp in range(4):
                out.append((sides[0][hp] & U32(0xFFFF)) | (sides[1][hp] << 16))
                out.append((sides[0][hp] >> 16) | (sides[1][hp] & U32(0xFFFF0000)))
            return out

        def pstage_m(o, m):
            p = _unpack(ptok_s[...])
            acc = None
            for k in range(DM // DH):
                blocks = [conv_block(o, m, 8 * k + b) for b in range(8)]
                w = jnp.concatenate([jnp.concatenate([blocks[b][h] for b in range(8)], axis=0)
                                     for h in range(8)], axis=1)
                for i in range(2):
                    w3_s[m][2 * o + i, pl.ds(k * 64, 64), :] = w[:, i * GW:(i + 1) * GW]
                r = _dot(p[:, k * DH:(k + 1) * DH], _unpack(w))
                acc = r if acc is None else acc + r
            r = _pack(acc)
            for i in range(2):
                for sg in range(NP):
                    ring_s[sg, 2 * o + i, m] = r[sg * 16:(sg + 1) * 16, i * GW:(i + 1) * GW]

        with jax.named_scope('P'):
            issue([cp_xh, cp3(0, 0), cp_m0] + [cp3(o, m) for o in range(2) for m in range(3) if o + m > 0])
            cp_xh.wait()
            for sg in range(NP):
                ptok_s[pl.ds(sg * 16, 16), :] = _pack(_ln(x0seg(sg)))

            def pstage(o, carry):
                @pl.when(o + 2 == NOCT)
                def _():
                    issue(cp_wo + [cp_wg, cp_wu, cp_wd, cp_xr])
                for m in range(3):
                    cp3(o, m).wait()
                    pstage_m(o, m)

                    @pl.when(o + 2 < NOCT)
                    def _():
                        cp3(o + 2, m).start()
                return carry
            lax.fori_loop(0, NOCT, pstage, 0)

        c1 = (DH ** -0.5) * LOG2E

        def make_mask(rows, tok_layers):
            row = lax.broadcasted_iota(jnp.int32, (rows, rows), 0)
            col = lax.broadcasted_iota(jnp.int32, (rows, rows), 1)

            def layer(i):
                lay = jnp.where(i < M, 0, 1)
                for b, l in enumerate(tok_layers):
                    lay = jnp.where(i >= MP + b * SEG, l, lay)
                return lay
            return (layer(row) == layer(col)) & ((row < MP) | (col < MP) | (row >= col))

        def split(r):
            return [r[:, j * DH:(j + 1) * DH] for j in range(HG)]

        def qkv_plain(hh):
            def get(g):
                return [[x.astype(BF16) for x in split(_dot(hh, _unpack(w3_s[m][g])))] for m in range(3)]
            return get

        def qkv_ring(hh, rd, wr):
            def get(g):
                out = []
                for m in range(3):
                    r = _dot(hh, _unpack(w3_s[m][g]))
                    old = split(_unpack(ring_s[rd, g, m]))
                    rs = split(r)
                    if wr is None:
                        out.append([jnp.concatenate([rs[j][:MP].astype(BF16), old[j], rs[j][MP:].astype(BF16)], axis=0)
                                    for j in range(HG)])
                    else:
                        ring_s[wr, g, m] = _pack(r[MP:])
                        out.append([jnp.concatenate([rs[j][:MP].astype(BF16), old[j]], axis=0) for j in range(HG)])
                return out
            return get

        def scores(q, k):
            return [lax.dot_general(q[j], k[j], (((1,), (1,)), ((), ())), preferred_element_type=F32)
                    for j in range(HG)]

        def softmax_pv(ss, v, mask):
            os_ = []
            for j in range(HG):
                s = jnp.where(mask, ss[j], NEG)
                mx = jnp.max(s, axis=-1, keepdims=True)
                e = jnp.exp2((s - mx) * c1)
                l = jnp.sum(e, axis=-1, keepdims=True)
                p = (e * pl.reciprocal(l, approx=True)).astype(BF16)
                os_.append(_dot(p, v[j]))
            return jnp.concatenate(os_, axis=1).astype(BF16)

        def wo(o, g, acc):
            r = _dot(o, _unpack(wo_s[pl.ds(g * (GW // 2), GW // 2), :]))
            return r if acc is None else acc + r

        def ffn_a(f, c0, c1_):
            gg = _dot(f, _unpack(wg_s[:, c0:c1_]))
            uu = _dot(f, _unpack(wu_s[:, c0:c1_]))
            return (uu * (0.5 * jnp.tanh(0.5 * gg) + 0.5)).astype(BF16)

        def ffn_b(a):
            return _dot(a, _unpack(wd_s[...]))

        def ffn32(r):
            return r + ffn_b(ffn_a(_ln(r).astype(BF16), 0, FF))

        def attention(get, mask, fillers, late_wo=None):
            qs, ss, oo = {}, {}, {}
            acc = None
            for i in range(NG + 3):
                if i < NG:
                    qs[i] = get(i)
                elif i - NG < len(fillers):
                    fillers[i - NG]()
                if 0 <= i - 2 < NG:
                    oo[i - 2] = softmax_pv(ss.pop(i - 2), qs.pop(i - 2)[2], mask)
                if 0 <= i - 1 < NG:
                    ss[i - 1] = scores(qs[i - 1][0], qs[i - 1][1])
                if 0 <= i - 3 < NG and late_wo is None:
                    acc = wo(oo.pop(i - 3), i - 3, acc)
            if late_wo is not None:
                acc = late_wo(oo)
            return acc

        def out_copy(seg, slot):
            return pltpu.make_async_copy(y_s.at[slot], y_hbm.at[pl.ds(seg * SEG, SEG)], osem.at[slot])

        def wait_y(yseg):
            @pl.when(yseg >= 2)
            def _():
                out_copy(yseg - 2, yseg % 2).wait()

        def emit_y(yseg, yv):
            yslot = yseg % 2
            y_s[yslot] = yv.astype(BF16)

            @pl.when(yseg >= 0)
            def _():
                out_copy(yseg, yslot).start()

        def mem_pair(t, l1_live=True):
            mem0 = mem0_ref[...].astype(F32)
            mem1 = acc_s[:M, :] if l1_live else jnp.zeros((M, DM), F32)
            mem2 = jnp.where(t <= D, mem0, acc_s[M:MP, :])
            return jnp.concatenate([mem1, mem2], axis=0).astype(BF16)

        def conv_all(src, dst):
            dst[...] = pltpu.bitcast(src[...], U32)

        cp_m0.wait()
        mem0 = mem0_ref[...].astype(F32)
        acc_s[...] = jnp.concatenate([mem0, mem0, jnp.zeros((2 * SEG, DM), F32)], axis=0)
        x2_s[XR2 - 1] = jnp.zeros((SEG, DM), F32)

        mask1 = make_mask(MP + SEG, [0])

        def pro(t, first):
            if not first:
                x1_s[t - 1] = x0seg(t - 1) + acc_s[MP:MP + SEG, :]
            hm = jnp.concatenate([acc_s[:M, :], mem0_ref[...].astype(F32)], axis=0).astype(BF16)
            hh = jnp.concatenate([hm, _ln(x0seg(t + NP)).astype(BF16)], axis=0)
            late = None
            if first:
                def late(oo):
                    acc = None
                    gpc = NG // WOC
                    for c in range(WOC):
                        cp_wo[c].wait()
                        for g in range(c * gpc, (c + 1) * gpc):
                            wov = pltpu.bitcast(wo_st[pl.ds(g * GW, GW), :], U32)
                            wo_s[pl.ds(g * (GW // 2), GW // 2), :] = wov
                            r = _dot(oo[g], _unpack(wov))
                            acc = r if acc is None else acc + r
                    return acc
            acc = attention(qkv_ring(hh, t, t + NP), mask1, [], late_wo=late)
            acc_s[:MP + SEG, :] = acc

        with jax.named_scope('PRO0'):
            pro(0, True)

        def pro_rest(t, carry):
            pro(t, False)
            return carry
        with jax.named_scope('PRO1'):
            lax.fori_loop(1, D, pro_rest, 0)
        with jax.named_scope('FFN0'):
            cp_wg.wait()
            cp_wu.wait()
            cp_wd.wait()
            r0 = x1_s[0]
            f0 = _ln(r0).astype(BF16)
            acts0 = []
            FC = 512
            for c0 in range(0, FF, FC):
                wgv = pltpu.bitcast(wg_st[:, c0:c0 + FC], U32)
                wuv = pltpu.bitcast(wu_st[:, c0:c0 + FC], U32)
                wg_s[:, c0:c0 + FC] = wgv
                wu_s[:, c0:c0 + FC] = wuv
                gg = _dot(f0, _unpack(wgv))
                uu = _dot(f0, _unpack(wuv))
                acts0.append((uu * (0.5 * jnp.tanh(0.5 * gg) + 0.5)).astype(BF16))
            x2 = r0
            for i, c0 in enumerate(range(0, FF, FC)):
                wdv = pltpu.bitcast(wd_st[c0:c0 + FC, :], U32)
                wd_s[c0 // 2:(c0 + FC) // 2, :] = wdv
                x2 = x2 + _dot(acts0[i], _unpack(wdv))
            x2_s[0] = x2
            htok_s[1] = _pack(_ln(x2))
            cp_xr.wait()

        mask2 = make_mask(MP + 2 * SEG, [0, 1])

        def step(t, carry, ringed):
            wait_y(t - D - 1)
            x1 = x0seg(t - 1) + acc_s[MP:MP + SEG, :]
            x3 = x2_s[(t - D - 1) % XR2] + acc_s[MP + SEG:, :]
            if ringed:
                get = qkv_ring(jnp.concatenate([mem_pair(t), _unpack(htok_s[1])], axis=0), t, None)
                first = t == D
                res = jnp.concatenate([jnp.where(first, x1_s[1], x1), jnp.where(first, x1, x3)], axis=0)
                aseg = jnp.where(first, 1, t - 1)
            else:
                get = qkv_plain(jnp.concatenate([mem_pair(t), _unpack(htok_s[0]), _unpack(htok_s[1])], axis=0))
                res = jnp.concatenate([x1, x3], axis=0)
                aseg = t - 1
            fin = _ln(res).astype(BF16)
            tok1 = _ln(x0seg(t + 1))
            acts = []
            fo = []
            fillers = [lambda: acts.append(ffn_a(fin, 0, FF // 2)),
                       lambda: acts.append(ffn_a(fin, FF // 2, FF)),
                       lambda: fo.append(ffn_b(jnp.concatenate(acts, axis=1)))]
            acc = attention(get, mask2, fillers)
            xo = res + fo[0]
            acc_s[...] = acc
            x2_s[aseg % XR2] = xo[:SEG]
            if ringed:
                x2_s[jnp.where(first, 2, XR2)] = xo[SEG:]
                tok2 = _ln(jnp.where(first, xo[:SEG], x2_s[(t + 1 - D) % XR2]))
            else:
                tok2 = _ln(x2_s[(t + 1 - D) % XR2])
            htok_s[0] = _pack(tok1)
            htok_s[1] = _pack(tok2)
            emit_y(t - D - 1, xo[SEG:])
            return carry
        with jax.named_scope('PDUAL'):
            lax.fori_loop(D, D + NP, functools.partial(step, ringed=True), 0)
        with jax.named_scope('MAIN'):
            lax.fori_loop(D + NP, NSEG, functools.partial(step, ringed=False), 0)

        mask3 = make_mask(MP + SEG, [1])

        def epi(t, carry):
            wait_y(t - D - 1)
            fres_s[0] = x0seg(t - 1) + acc_s[MP:MP + SEG, :]
            fres_s[1] = x2_s[(t - D - 1) % XR2] + acc_s[MP + SEG:, :]

            @pl.when(t < NSEG + D)
            def _():
                hh = jnp.concatenate([mem_pair(t, l1_live=False), _unpack(htok_s[1])], axis=0)
                acc = attention(qkv_plain(hh), mask3, [])
                acc_s[:MP, :] = acc[:MP]
                acc_s[MP + SEG:, :] = acc[MP:]

            def f(w, c):
                xo = ffn32(fres_s[w])

                @pl.when(w == 0)
                def _():
                    x2_s[(NSEG - 1) % XR2] = xo

                @pl.when(w == 1)
                def _():
                    emit_y(t - D - 1, xo)
                return c
            lax.fori_loop(jnp.where(t == NSEG, 0, 1), 2, f, 0)
            htok_s[1] = _pack(_ln(x2_s[(t + 1 - D) % XR2]))
            return carry
        with jax.named_scope('EPI'):
            lax.fori_loop(NSEG, NSEG + D + 1, epi, 0)
        out_copy(NSEG - 2, 0).wait()
        out_copy(NSEG - 1, 1).wait()

    def run(A_x, A_mem0, A_Wq, A_Wk, A_Wv, A_Wo, A_seg_len, B_x, B_w_gate, B_w_up, B_w_down):
        any_spec = pl.BlockSpec(memory_space=pl.ANY)
        out = pl.pallas_call(
            kernel,
            out_shape=jax.ShapeDtypeStruct((S, DM), BF16),
            in_specs=[any_spec] * 9,
            out_specs=any_spec,
            scratch_shapes=[
                pltpu.VMEM((NG, DM // 2, GW), U32),
                pltpu.VMEM((NG, DM // 2, GW), U32),
                pltpu.VMEM((NG, DM // 2, GW), U32),
                pltpu.VMEM((H * DH // 2, DM), U32),
                pltpu.VMEM((DM // 2, FF), U32),
                pltpu.VMEM((DM // 2, FF), U32),
                pltpu.VMEM((FF // 2, DM), U32),
                pltpu.VMEM((2, 3, DM, 8, DH), BF16),
                pltpu.VMEM((H * DH, DM), BF16),
                pltpu.VMEM((DM, FF), BF16),
                pltpu.VMEM((DM, FF), BF16),
                pltpu.VMEM((FF, DM), BF16),
                pltpu.VMEM((S, DM), BF16),
                pltpu.VMEM((M, DM), BF16),
                pltpu.VMEM((NP * SEG // 2, DM), U32),
                pltpu.VMEM((R, NG, 3, SEG // 2, GW), U32),
                pltpu.VMEM((2, SEG // 2, DM), U32),
                pltpu.VMEM((MP + 2 * SEG, DM), F32),
                pltpu.VMEM((2, SEG, DM), F32),
                pltpu.VMEM((XR2 + 1, SEG, DM), F32),
                pltpu.VMEM((2, SEG, DM), F32),
                pltpu.VMEM((2, SEG, DM), BF16),
                pltpu.SemaphoreType.DMA((2, 3)),
                pltpu.SemaphoreType.DMA((6 + WOC,)),
                pltpu.SemaphoreType.DMA((2,)),
            ],
            compiler_params=pltpu.CompilerParams(vmem_limit_bytes=124 * 1024 * 1024, disable_bounds_checks=bool(NOBC)),
            name="memtr",
        )(A_x.reshape(S, DM), A_mem0.reshape(M, DM), A_Wq, A_Wk, A_Wv, A_Wo.reshape(H * DH, DM),
          B_w_gate, B_w_up, B_w_down)
        return out.reshape(1, S, DM)
    return run


_run = _make()


@functools.partial(jax.jit, static_argnames=("A_seg_len",))
def pallas_interleave_layers__memory_aug_recurrent_mem_tr__glu_gated_glu__prompt_kernel(
    A_x, A_mem0, A_Wq, A_Wk, A_Wv, A_Wo, A_seg_len, B_x, B_w_gate, B_w_up, B_w_down,
):
    assert A_seg_len == SEG
    assert A_x.shape == (1, S, DM) and A_mem0.shape == (1, M, DM)
    assert A_Wq.shape == (DM, H, DH) and A_Wo.shape == (H, DH, DM)
    assert B_w_gate.shape == (DM, FF) and B_w_down.shape == (FF, DM)
    return _run(A_x, A_mem0, A_Wq, A_Wk, A_Wv, A_Wo, A_seg_len, B_x, B_w_gate, B_w_up, B_w_down)
```

```python
import functools
import jax
import jax.numpy as jnp
from jax import lax
from jax.experimental import pallas as pl
from jax.experimental.pallas import tpu as pltpu

S, DM, H, DH, M, SEG, FF = 2048, 1024, 32, 128, 8, 32, 3584
NSEG = S // SEG
MP = 2 * M
U32 = jnp.uint32
BF16 = jnp.bfloat16
F32 = jnp.float32
EPS = 1e-5
NEG = -1e9
LOG2E = 1.4426950408889634


def _pack(x):
    return pltpu.bitcast(x.astype(BF16), U32)


def _unpack(x):
    return pltpu.bitcast(x, BF16)


def _ln(x):
    m = jnp.mean(x, axis=-1, keepdims=True)
    xc = x - m
    v = jnp.mean(xc * xc, axis=-1, keepdims=True)
    return xc * lax.rsqrt(v + EPS)


def _glu(g, u):
    return u * pl.reciprocal(1.0 + jnp.exp2(g * (-LOG2E)), approx=True)


def _dot(a, b):
    return jnp.dot(a, b, preferred_element_type=F32)


def _make(D=3, NP=11, NOBC=0):
    NG = 8
    HG = H // NG
    GW = HG * DH
    NOCT = H // 8
    WOC = 4
    R = NP + D
    XR2 = 4
    assert D == 3
    XH = NP + D + 1

    def kernel(x_hbm, mem0_hbm, wq_hbm, wk_hbm, wv_hbm, wo_hbm, wg_hbm, wu_hbm, wd_hbm,
               y_hbm,
               wq_s, wk_s, wv_s, wo_s, wg_s, wu_s, wd_s, st3_s, wo_st, wg_st, wu_st, wd_st,
               x0_s, mem0_ref, ptok_s, ring_s, htok_s, acc_s, x1_s, x2_s, fres_s, y_s, sem3, semw, osem):
        srcs = [wq_hbm, wk_hbm, wv_hbm]
        w3_s = [wq_s, wk_s, wv_s]

        def cp3(o, m):
            return pltpu.make_async_copy(srcs[m].at[:, pl.ds(pl.multiple_of(o * 8, 8), 8), :],
                                         st3_s.at[o % 2, m], sem3.at[o % 2, m])
        XR = XH * SEG
        cp_xh = pltpu.make_async_copy(x_hbm.at[pl.ds(0, XR)], x0_s.at[pl.ds(0, XR)], semw.at[0])
        cp_xr = pltpu.make_async_copy(x_hbm.at[pl.ds(XR, S - XR)], x0_s.at[pl.ds(XR, S - XR)], semw.at[1])
        cp_m0 = pltpu.make_async_copy(mem0_hbm, mem0_ref, semw.at[5 + WOC])
        WOR = H * DH // WOC
        cp_wo = [pltpu.make_async_copy(wo_hbm.at[pl.ds(c * WOR, WOR)], wo_st.at[pl.ds(c * WOR, WOR)], semw.at[2 + c])
                 for c in range(WOC)]
        cp_wg = pltpu.make_async_copy(wg_hbm, wg_st, semw.at[2 + WOC])
        cp_wu = pltpu.make_async_copy(wu_hbm, wu_st, semw.at[3 + WOC])
        cp_wd = pltpu.make_async_copy(wd_hbm, wd_st, semw.at[4 + WOC])

        def issue(descs):
            def body(i, c):
                for k, d in enumerate(descs):
                    pl.when(i == k)(d.start)
                return c
            lax.fori_loop(0, len(descs), body, 0)

        def x0seg(i):
            i = jnp.clip(i, 0, NSEG - 1)
            return x0_s[pl.ds(pl.multiple_of(i * SEG, SEG), SEG), :].astype(F32)

        sub8 = lax.broadcasted_iota(jnp.int32, (8, DH), 0)

        def conv_block(o, m, b):
            s32 = pltpu.bitcast(st3_s[o % 2, m, pl.ds(b * 16, 16)], U32).reshape(8, 2, 4, DH)
            sides = []
            for par in range(2):
                P = [jnp.concatenate([s32[k, par], s32[k + 4, par]], axis=0) for k in range(4)]
                for dist in (1, 2):
                    msk = (sub8 & dist) == 0
                    Q = list(P)
                    for k in range(4):
                        if k & dist == 0:
                            Q[k] = jnp.where(msk, P[k], pltpu.roll(P[k + dist], dist, 0))
                            Q[k + dist] = jnp.where(msk, pltpu.roll(P[k], 8 - dist, 0), P[k + dist])
                    P = Q
                sides.append(P)
            out = []
            for hp in range(4):
                out.append((sides[0][hp] & U32(0xFFFF)) | (sides[1][hp] << 16))
                out.append((sides[0][hp] >> 16) | (sides[1][hp] & U32(0xFFFF0000)))
            return out

        def pstage_m(o, m):
            p = _unpack(ptok_s[...])
            acc = None
            for k in range(DM // DH):
                blocks = [conv_block(o, m, 8 * k + b) for b in range(8)]
                w = jnp.concatenate([jnp.concatenate([blocks[b][h] for b in range(8)], axis=0)
                                     for h in range(8)], axis=1)
                for i in range(2):
                    w3_s[m][2 * o + i, pl.ds(k * 64, 64), :] = w[:, i * GW:(i + 1) * GW]
                r = _dot(p[:, k * DH:(k + 1) * DH], _unpack(w))
                acc = r if acc is None else acc + r
            r = _pack(acc)
            for i in range(2):
                for sg in range(NP):
                    ring_s[sg, 2 * o + i, m] = r[sg * 16:(sg + 1) * 16, i * GW:(i + 1) * GW]

        with jax.named_scope('P'):
            issue([cp_xh, cp3(0, 0), cp_m0] + [cp3(o, m) for o in range(2) for m in range(3) if o + m > 0])
            cp_xh.wait()
            for sg in range(NP):
                ptok_s[pl.ds(sg * 16, 16), :] = _pack(_ln(x0seg(sg)))

            def pstage(o, carry):
                @pl.when(o + 2 == NOCT)
                def _():
                    issue(cp_wo + [cp_wg, cp_wu, cp_wd, cp_xr])
                for m in range(3):
                    cp3(o, m).wait()
                    pstage_m(o, m)

                    @pl.when(o + 2 < NOCT)
                    def _():
                        cp3(o + 2, m).start()
                return carry
            lax.fori_loop(0, NOCT, pstage, 0)

        c1 = (DH ** -0.5) * LOG2E

        def make_mask(rows, tok_layers):
            row = lax.broadcasted_iota(jnp.int32, (rows, rows), 0)
            col = lax.broadcasted_iota(jnp.int32, (rows, rows), 1)

            def layer(i):
                lay = jnp.where(i < M, 0, 1)
                for b, l in enumerate(tok_layers):
                    lay = jnp.where(i >= MP + b * SEG, l, lay)
                return lay
            return (layer(row) == layer(col)) & ((row < MP) | (col < MP) | (row >= col))

        def split(r):
            return [r[:, j * DH:(j + 1) * DH] for j in range(HG)]

        def qkv_plain(hh):
            def get(g):
                return [[x.astype(BF16) for x in split(_dot(hh, _unpack(w3_s[m][g])))] for m in range(3)]
            return get

        def qkv_ring(hh, rd, wr):
            def get(g):
                out = []
                for m in range(3):
                    r = _dot(hh, _unpack(w3_s[m][g]))
                    old = split(_unpack(ring_s[rd, g, m]))
                    rs = split(r)
                    if wr is None:
                        out.append([jnp.concatenate([rs[j][:MP].astype(BF16), old[j], rs[j][MP:].astype(BF16)], axis=0)
                                    for j in range(HG)])
                    else:
                        ring_s[wr, g, m] = _pack(r[MP:])
                        out.append([jnp.concatenate([rs[j][:MP].astype(BF16), old[j]], axis=0) for j in range(HG)])
                return out
            return get

        def scores(q, k):
            return [lax.dot_general(q[j], k[j], (((1,), (1,)), ((), ())), preferred_element_type=F32)
                    for j in range(HG)]

        def softmax_pv(ss, v, mask):
            os_ = []
            for j in range(HG):
                s = jnp.where(mask, ss[j], NEG)
                mx = jnp.max(s, axis=-1, keepdims=True)
                e = jnp.exp2((s - mx) * c1)
                l = jnp.sum(e, axis=-1, keepdims=True)
                p = (e * pl.reciprocal(l, approx=True)).astype(BF16)
                os_.append(_dot(p, v[j]))
            return jnp.concatenate(os_, axis=1).astype(BF16)

        def wo(o, g, acc):
            r = _dot(o, _unpack(wo_s[pl.ds(g * (GW // 2), GW // 2), :]))
            return r if acc is None else acc + r

        def ffn_a(f, c0, c1_):
            gg = _dot(f, _unpack(wg_s[:, c0:c1_]))
            uu = _dot(f, _unpack(wu_s[:, c0:c1_]))
            return _glu(gg, uu).astype(BF16)

        def ffn_b(a):
            return _dot(a, _unpack(wd_s[...]))

        def ffn32(r):
            return r + ffn_b(ffn_a(_ln(r).astype(BF16), 0, FF))

        def attention(get, mask, fillers, late_wo=None):
            qs, ss, oo = {}, {}, {}
            acc = None
            for i in range(NG + 3):
                if i < NG:
                    qs[i] = get(i)
                elif i - NG < len(fillers):
                    fillers[i - NG]()
                if 0 <= i - 2 < NG:
                    oo[i - 2] = softmax_pv(ss.pop(i - 2), qs.pop(i - 2)[2], mask)
                if 0 <= i - 1 < NG:
                    ss[i - 1] = scores(qs[i - 1][0], qs[i - 1][1])
                if 0 <= i - 3 < NG and late_wo is None:
                    acc = wo(oo.pop(i - 3), i - 3, acc)
            if late_wo is not None:
                acc = late_wo(oo)
            return acc

        def out_copy(seg, slot):
            return pltpu.make_async_copy(y_s.at[slot], y_hbm.at[pl.ds(seg * SEG, SEG)], osem.at[slot])

        def wait_y(yseg):
            @pl.when(yseg >= 2)
            def _():
                out_copy(yseg - 2, yseg % 2).wait()

        def emit_y(yseg, yv):
            yslot = yseg % 2
            y_s[yslot] = yv.astype(BF16)

            @pl.when(yseg >= 0)
            def _():
                out_copy(yseg, yslot).start()

        def mem_pair(t, l1_live=True):
            mem0 = mem0_ref[...].astype(F32)
            mem1 = acc_s[:M, :] if l1_live else jnp.zeros((M, DM), F32)
            mem2 = jnp.where(t <= D, mem0, acc_s[M:MP, :])
            return jnp.concatenate([mem1, mem2], axis=0).astype(BF16)

        def conv_all(src, dst):
            dst[...] = pltpu.bitcast(src[...], U32)

        cp_m0.wait()
        mem0 = mem0_ref[...].astype(F32)
        acc_s[...] = jnp.concatenate([mem0, mem0, jnp.zeros((2 * SEG, DM), F32)], axis=0)
        x2_s[XR2 - 1] = jnp.zeros((SEG, DM), F32)

        mask1 = make_mask(MP + SEG, [0])

        def pro(t, first):
            if not first:
                x1_s[t - 1] = x0seg(t - 1) + acc_s[MP:MP + SEG, :]
            hm = jnp.concatenate([acc_s[:M, :], mem0_ref[...].astype(F32)], axis=0).astype(BF16)
            hh = jnp.concatenate([hm, _ln(x0seg(t + NP)).astype(BF16)], axis=0)
            late = None
            if first:
                def late(oo):
                    acc = None
                    gpc = NG // WOC
                    for c in range(WOC):
                        cp_wo[c].wait()
                        for g in range(c * gpc, (c + 1) * gpc):
                            wov = pltpu.bitcast(wo_st[pl.ds(g * GW, GW), :], U32)
                            wo_s[pl.ds(g * (GW // 2), GW // 2), :] = wov
                            r = _dot(oo[g], _unpack(wov))
                            acc = r if acc is None else acc + r
                    return acc
            acc = attention(qkv_ring(hh, t, t + NP), mask1, [], late_wo=late)
            acc_s[:MP + SEG, :] = acc

        with jax.named_scope('PRO0'):
            pro(0, True)

        def pro_rest(t, carry):
            pro(t, False)
            return carry
        with jax.named_scope('PRO1'):
            lax.fori_loop(1, D, pro_rest, 0)
        with jax.named_scope('FFN0'):
            cp_wg.wait()
            cp_wu.wait()
            cp_wd.wait()
            r0 = x1_s[0]
            f0 = _ln(r0).astype(BF16)
            acts0 = []
            FC = 512
            for c0 in range(0, FF, FC):
                wgv = pltpu.bitcast(wg_st[:, c0:c0 + FC], U32)
                wuv = pltpu.bitcast(wu_st[:, c0:c0 + FC], U32)
                wg_s[:, c0:c0 + FC] = wgv
                wu_s[:, c0:c0 + FC] = wuv
                gg = _dot(f0, _unpack(wgv))
                uu = _dot(f0, _unpack(wuv))
                acts0.append(_glu(gg, uu).astype(BF16))
            x2 = r0
            for i, c0 in enumerate(range(0, FF, FC)):
                wdv = pltpu.bitcast(wd_st[c0:c0 + FC, :], U32)
                wd_s[c0 // 2:(c0 + FC) // 2, :] = wdv
                x2 = x2 + _dot(acts0[i], _unpack(wdv))
            x2_s[0] = x2
            htok_s[1] = _pack(_ln(x2))
            cp_xr.wait()

        mask2 = make_mask(MP + 2 * SEG, [0, 1])

        def step(t, carry, ringed):
            wait_y(t - D - 1)
            x1 = x0seg(t - 1) + acc_s[MP:MP + SEG, :]
            x3 = x2_s[(t - D - 1) % XR2] + acc_s[MP + SEG:, :]
            if ringed:
                get = qkv_ring(jnp.concatenate([mem_pair(t), _unpack(htok_s[1])], axis=0), t, None)
                first = t == D
                res = jnp.concatenate([jnp.where(first, x1_s[1], x1), jnp.where(first, x1, x3)], axis=0)
                aseg = jnp.where(first, 1, t - 1)
            else:
                get = qkv_plain(jnp.concatenate([mem_pair(t), _unpack(htok_s[0]), _unpack(htok_s[1])], axis=0))
                res = jnp.concatenate([x1, x3], axis=0)
                aseg = t - 1
            fin = _ln(res).astype(BF16)
            tok1 = _ln(x0seg(t + 1))
            acts = []
            fo = []
            fillers = [lambda: acts.append(ffn_a(fin, 0, FF // 2)),
                       lambda: acts.append(ffn_a(fin, FF // 2, FF)),
                       lambda: fo.append(ffn_b(jnp.concatenate(acts, axis=1)))]
            acc = attention(get, mask2, fillers)
            xo = res + fo[0]
            acc_s[...] = acc
            x2_s[aseg % XR2] = xo[:SEG]
            if ringed:
                x2_s[jnp.where(first, 2, XR2)] = xo[SEG:]
                tok2 = _ln(jnp.where(first, xo[:SEG], x2_s[(t + 1 - D) % XR2]))
            else:
                tok2 = _ln(x2_s[(t + 1 - D) % XR2])
            htok_s[0] = _pack(tok1)
            htok_s[1] = _pack(tok2)
            emit_y(t - D - 1, xo[SEG:])
            return carry
        with jax.named_scope('PDUAL'):
            lax.fori_loop(D, D + NP, functools.partial(step, ringed=True), 0)
        with jax.named_scope('MAIN'):
            lax.fori_loop(D + NP, NSEG, functools.partial(step, ringed=False), 0)

        mask3 = make_mask(MP + SEG, [1])

        def epi(t, carry):
            wait_y(t - D - 1)
            fres_s[0] = x0seg(t - 1) + acc_s[MP:MP + SEG, :]
            fres_s[1] = x2_s[(t - D - 1) % XR2] + acc_s[MP + SEG:, :]

            @pl.when(t < NSEG + D)
            def _():
                hh = jnp.concatenate([mem_pair(t, l1_live=False), _unpack(htok_s[1])], axis=0)
                acc = attention(qkv_plain(hh), mask3, [])
                acc_s[:MP, :] = acc[:MP]
                acc_s[MP + SEG:, :] = acc[MP:]

            def f(w, c):
                xo = ffn32(fres_s[w])

                @pl.when(w == 0)
                def _():
                    x2_s[(NSEG - 1) % XR2] = xo

                @pl.when(w == 1)
                def _():
                    emit_y(t - D - 1, xo)
                return c
            lax.fori_loop(jnp.where(t == NSEG, 0, 1), 2, f, 0)
            htok_s[1] = _pack(_ln(x2_s[(t + 1 - D) % XR2]))
            return carry
        with jax.named_scope('EPI'):
            lax.fori_loop(NSEG, NSEG + D + 1, epi, 0)
        out_copy(NSEG - 2, 0).wait()
        out_copy(NSEG - 1, 1).wait()

    def run(A_x, A_mem0, A_Wq, A_Wk, A_Wv, A_Wo, A_seg_len, B_x, B_w_gate, B_w_up, B_w_down):
        any_spec = pl.BlockSpec(memory_space=pl.ANY)
        out = pl.pallas_call(
            kernel,
            out_shape=jax.ShapeDtypeStruct((S, DM), BF16),
            in_specs=[any_spec] * 9,
            out_specs=any_spec,
            scratch_shapes=[
                pltpu.VMEM((NG, DM // 2, GW), U32),
                pltpu.VMEM((NG, DM // 2, GW), U32),
                pltpu.VMEM((NG, DM // 2, GW), U32),
                pltpu.VMEM((H * DH // 2, DM), U32),
                pltpu.VMEM((DM // 2, FF), U32),
                pltpu.VMEM((DM // 2, FF), U32),
                pltpu.VMEM((FF // 2, DM), U32),
                pltpu.VMEM((2, 3, DM, 8, DH), BF16),
                pltpu.VMEM((H * DH, DM), BF16),
                pltpu.VMEM((DM, FF), BF16),
                pltpu.VMEM((DM, FF), BF16),
                pltpu.VMEM((FF, DM), BF16),
                pltpu.VMEM((S, DM), BF16),
                pltpu.VMEM((M, DM), BF16),
                pltpu.VMEM((NP * SEG // 2, DM), U32),
                pltpu.VMEM((R, NG, 3, SEG // 2, GW), U32),
                pltpu.VMEM((2, SEG // 2, DM), U32),
                pltpu.VMEM((MP + 2 * SEG, DM), F32),
                pltpu.VMEM((2, SEG, DM), F32),
                pltpu.VMEM((XR2 + 1, SEG, DM), F32),
                pltpu.VMEM((2, SEG, DM), F32),
                pltpu.VMEM((2, SEG, DM), BF16),
                pltpu.SemaphoreType.DMA((2, 3)),
                pltpu.SemaphoreType.DMA((6 + WOC,)),
                pltpu.SemaphoreType.DMA((2,)),
            ],
            compiler_params=pltpu.CompilerParams(vmem_limit_bytes=124 * 1024 * 1024, disable_bounds_checks=bool(NOBC)),
            name="memtr",
        )(A_x.reshape(S, DM), A_mem0.reshape(M, DM), A_Wq, A_Wk, A_Wv, A_Wo.reshape(H * DH, DM),
          B_w_gate, B_w_up, B_w_down)
        return out.reshape(1, S, DM)
    return run


_run = _make()


@functools.partial(jax.jit, static_argnames=("A_seg_len",))
def pallas_interleave_layers__memory_aug_recurrent_mem_tr__glu_gated_glu__prompt_kernel(
    A_x, A_mem0, A_Wq, A_Wk, A_Wv, A_Wo, A_seg_len, B_x, B_w_gate, B_w_up, B_w_down,
):
    assert A_seg_len == SEG
    assert A_x.shape == (1, S, DM) and A_mem0.shape == (1, M, DM)
    assert A_Wq.shape == (DM, H, DH) and A_Wo.shape == (H, DH, DM)
    assert B_w_gate.shape == (DM, FF) and B_w_down.shape == (FF, DM)
    return _run(A_x, A_mem0, A_Wq, A_Wk, A_Wv, A_Wo, A_seg_len, B_x, B_w_gate, B_w_up, B_w_down)
```

```python
import functools
import jax
import jax.numpy as jnp
from jax import lax
from jax.experimental import pallas as pl
from jax.experimental.pallas import tpu as pltpu

S, DM, H, DH, M, SEG, FF = 2048, 1024, 32, 128, 8, 32, 3584
NSEG = S // SEG
MP = 2 * M
U32 = jnp.uint32
BF16 = jnp.bfloat16
F32 = jnp.float32
EPS = 1e-5
NEG = -1e9
LOG2E = 1.4426950408889634


def _pack(x):
    return pltpu.bitcast(x.astype(BF16), U32)


def _unpack(x):
    return pltpu.bitcast(x, BF16)


def _ln(x):
    m = jnp.mean(x, axis=-1, keepdims=True)
    xc = x - m
    v = jnp.mean(xc * xc, axis=-1, keepdims=True)
    return xc * lax.rsqrt(v + EPS)


def _glu(g, u):
    return u * pl.reciprocal(1.0 + jnp.exp2(g * (-LOG2E)), approx=True)


def _dot(a, b):
    return jnp.dot(a, b, preferred_element_type=F32)


def _make(D=3, NP=11, NOBC=0):
    NG = 8
    HG = H // NG
    GW = HG * DH
    NOCT = H // 8
    WOC = 4
    R = NP + D
    XR2 = 4
    assert D == 3
    XH = NP + D + 1

    def kernel(x_hbm, mem0_hbm, wq_hbm, wk_hbm, wv_hbm, wo_hbm, wg_hbm, wu_hbm, wd_hbm,
               y_hbm,
               wq_s, wk_s, wv_s, wo_s, wg_s, wu_s, wd_s, st3_s, wo_st, wg_st, wu_st, wd_st,
               x0_s, mem0_ref, ptok_s, ring_s, htok_s, acc_s, x1_s, x2_s, fres_s, y_s, sem3, semw, osem):
        srcs = [wq_hbm, wk_hbm, wv_hbm]
        w3_s = [wq_s, wk_s, wv_s]

        def cp3(o, m):
            return pltpu.make_async_copy(srcs[m].at[:, pl.ds(pl.multiple_of(o * 8, 8), 8), :],
                                         st3_s.at[o % 2, m], sem3.at[o % 2, m])
        XR = XH * SEG
        XA = NP * SEG
        cp_xh = pltpu.make_async_copy(x_hbm.at[pl.ds(0, XA)], x0_s.at[pl.ds(0, XA)], semw.at[0])
        cp_xb = pltpu.make_async_copy(x_hbm.at[pl.ds(XA, XR - XA)], x0_s.at[pl.ds(XA, XR - XA)], semw.at[6 + WOC])
        cp_xr = pltpu.make_async_copy(x_hbm.at[pl.ds(XR, S - XR)], x0_s.at[pl.ds(XR, S - XR)], semw.at[1])
        cp_m0 = pltpu.make_async_copy(mem0_hbm, mem0_ref, semw.at[5 + WOC])
        WOR = H * DH // WOC
        cp_wo = [pltpu.make_async_copy(wo_hbm.at[pl.ds(c * WOR, WOR)], wo_st.at[pl.ds(c * WOR, WOR)], semw.at[2 + c])
                 for c in range(WOC)]
        cp_wg = pltpu.make_async_copy(wg_hbm, wg_st, semw.at[2 + WOC])
        cp_wu = pltpu.make_async_copy(wu_hbm, wu_st, semw.at[3 + WOC])
        cp_wd = pltpu.make_async_copy(wd_hbm, wd_st, semw.at[4 + WOC])

        def issue(descs):
            def body(i, c):
                for k, d in enumerate(descs):
                    pl.when(i == k)(d.start)
                return c
            lax.fori_loop(0, len(descs), body, 0)

        def x0seg(i):
            i = jnp.clip(i, 0, NSEG - 1)
            return x0_s[pl.ds(pl.multiple_of(i * SEG, SEG), SEG), :].astype(F32)

        sub8 = lax.broadcasted_iota(jnp.int32, (8, DH), 0)

        def conv_block(o, m, b):
            s32 = pltpu.bitcast(st3_s[o % 2, m, pl.ds(b * 16, 16)], U32).reshape(8, 2, 4, DH)
            sides = []
            for par in range(2):
                P = [jnp.concatenate([s32[k, par], s32[k + 4, par]], axis=0) for k in range(4)]
                for dist in (1, 2):
                    msk = (sub8 & dist) == 0
                    Q = list(P)
                    for k in range(4):
                        if k & dist == 0:
                            Q[k] = jnp.where(msk, P[k], pltpu.roll(P[k + dist], dist, 0))
                            Q[k + dist] = jnp.where(msk, pltpu.roll(P[k], 8 - dist, 0), P[k + dist])
                    P = Q
                sides.append(P)
            out = []
            for hp in range(4):
                out.append((sides[0][hp] & U32(0xFFFF)) | (sides[1][hp] << 16))
                out.append((sides[0][hp] >> 16) | (sides[1][hp] & U32(0xFFFF0000)))
            return out

        def pstage_m(o, m):
            p = _unpack(ptok_s[...])
            acc = None
            for k in range(DM // DH):
                blocks = [conv_block(o, m, 8 * k + b) for b in range(8)]
                w = jnp.concatenate([jnp.concatenate([blocks[b][h] for b in range(8)], axis=0)
                                     for h in range(8)], axis=1)
                for i in range(2):
                    w3_s[m][2 * o + i, pl.ds(k * 64, 64), :] = w[:, i * GW:(i + 1) * GW]
                r = _dot(p[:, k * DH:(k + 1) * DH], _unpack(w))
                acc = r if acc is None else acc + r
            r = _pack(acc)
            for i in range(2):
                for sg in range(NP):
                    ring_s[sg, 2 * o + i, m] = r[sg * 16:(sg + 1) * 16, i * GW:(i + 1) * GW]

        with jax.named_scope('P'):
            issue([cp_xh, cp3(0, 0), cp3(0, 1), cp_xb, cp_m0] + [cp3(o, m) for o in range(2) for m in range(3) if 3 * o + m > 1])
            cp_xh.wait()
            for sg in range(NP):
                ptok_s[pl.ds(sg * 16, 16), :] = _pack(_ln(x0seg(sg)))

            def pstage(o, carry):
                @pl.when(o + 2 == NOCT)
                def _():
                    issue(cp_wo + [cp_wg, cp_wu, cp_wd, cp_xr])
                for m in range(3):
                    cp3(o, m).wait()
                    pstage_m(o, m)

                    @pl.when(o + 2 < NOCT)
                    def _():
                        cp3(o + 2, m).start()
                return carry
            lax.fori_loop(0, NOCT, pstage, 0)

        c1 = (DH ** -0.5) * LOG2E

        def make_mask(rows, tok_layers):
            row = lax.broadcasted_iota(jnp.int32, (rows, rows), 0)
            col = lax.broadcasted_iota(jnp.int32, (rows, rows), 1)

            def layer(i):
                lay = jnp.where(i < M, 0, 1)
                for b, l in enumerate(tok_layers):
                    lay = jnp.where(i >= MP + b * SEG, l, lay)
                return lay
            return (layer(row) == layer(col)) & ((row < MP) | (col < MP) | (row >= col))

        def split(r):
            return [r[:, j * DH:(j + 1) * DH] for j in range(HG)]

        def qkv_plain(hh):
            def get(g):
                return [[x.astype(BF16) for x in split(_dot(hh, _unpack(w3_s[m][g])))] for m in range(3)]
            return get

        def qkv_ring(hh, rd, wr):
            def get(g):
                out = []
                for m in range(3):
                    r = _dot(hh, _unpack(w3_s[m][g]))
                    old = split(_unpack(ring_s[rd, g, m]))
                    rs = split(r)
                    if wr is None:
                        out.append([jnp.concatenate([rs[j][:MP].astype(BF16), old[j], rs[j][MP:].astype(BF16)], axis=0)
                                    for j in range(HG)])
                    else:
                        ring_s[wr, g, m] = _pack(r[MP:])
                        out.append([jnp.concatenate([rs[j][:MP].astype(BF16), old[j]], axis=0) for j in range(HG)])
                return out
            return get

        def scores(q, k):
            return [lax.dot_general(q[j], k[j], (((1,), (1,)), ((), ())), preferred_element_type=F32)
                    for j in range(HG)]

        def softmax_pv(ss, v, mask):
            os_ = []
            for j in range(HG):
                s = jnp.where(mask, ss[j], NEG)
                mx = jnp.max(s, axis=-1, keepdims=True)
                e = jnp.exp2((s - mx) * c1)
                l = jnp.sum(e, axis=-1, keepdims=True)
                p = (e * pl.reciprocal(l, approx=True)).astype(BF16)
                os_.append(_dot(p, v[j]))
            return jnp.concatenate(os_, axis=1).astype(BF16)

        def wo(o, g, acc):
            r = _dot(o, _unpack(wo_s[pl.ds(g * (GW // 2), GW // 2), :]))
            return r if acc is None else acc + r

        def ffn_a(f, c0, c1_):
            gg = _dot(f, _unpack(wg_s[:, c0:c1_]))
            uu = _dot(f, _unpack(wu_s[:, c0:c1_]))
            return _glu(gg, uu).astype(BF16)

        def ffn_b(a):
            return _dot(a, _unpack(wd_s[...]))

        def ffn32(r):
            return r + ffn_b(ffn_a(_ln(r).astype(BF16), 0, FF))

        def attention(get, mask, fillers, wo=wo):
            qs, ss, oo = {}, {}, {}
            acc = None
            for i in range(NG + 3):
                if i < NG:
                    qs[i] = get(i)
                elif i - NG < len(fillers):
                    fillers[i - NG]()
                if 0 <= i - 2 < NG:
                    oo[i - 2] = softmax_pv(ss.pop(i - 2), qs.pop(i - 2)[2], mask)
                if 0 <= i - 1 < NG:
                    ss[i - 1] = scores(qs[i - 1][0], qs[i - 1][1])
                if 0 <= i - 3 < NG:
                    acc = wo(oo.pop(i - 3), i - 3, acc)
            return acc

        def out_copy(seg, slot):
            return pltpu.make_async_copy(y_s.at[slot], y_hbm.at[pl.ds(seg * SEG, SEG)], osem.at[slot])

        def wait_y(yseg):
            @pl.when(yseg >= 2)
            def _():
                out_copy(yseg - 2, yseg % 2).wait()

        def emit_y(yseg, yv):
            yslot = yseg % 2
            y_s[yslot] = yv.astype(BF16)

            @pl.when(yseg >= 0)
            def _():
                out_copy(yseg, yslot).start()

        def mem_pair(t, l1_live=True):
            mem0 = mem0_ref[...].astype(F32)
            mem1 = acc_s[:M, :] if l1_live else jnp.zeros((M, DM), F32)
            mem2 = jnp.where(t <= D, mem0, acc_s[M:MP, :])
            return jnp.concatenate([mem1, mem2], axis=0).astype(BF16)

        def conv_all(src, dst):
            dst[...] = pltpu.bitcast(src[...], U32)

        cp_m0.wait()
        cp_xb.wait()
        mem0 = mem0_ref[...].astype(F32)
        acc_s[...] = jnp.concatenate([mem0, mem0, jnp.zeros((2 * SEG, DM), F32)], axis=0)
        x2_s[XR2 - 1] = jnp.zeros((SEG, DM), F32)

        mask1 = make_mask(MP + SEG, [0])

        def pro(t, first):
            if not first:
                x1_s[t - 1] = x0seg(t - 1) + acc_s[MP:MP + SEG, :]
            hm = jnp.concatenate([acc_s[:M, :], mem0_ref[...].astype(F32)], axis=0).astype(BF16)
            hh = jnp.concatenate([hm, _ln(x0seg(t + NP)).astype(BF16)], axis=0)
            if first:
                for c in cp_wo:
                    c.wait()

                def wo_first(o, g, acc):
                    wov = pltpu.bitcast(wo_st[pl.ds(g * GW, GW), :], U32)
                    wo_s[pl.ds(g * (GW // 2), GW // 2), :] = wov
                    r = _dot(o, _unpack(wov))
                    return r if acc is None else acc + r
            acc = attention(qkv_ring(hh, t, t + NP), mask1, [], wo=wo_first if first else wo)
            acc_s[:MP + SEG, :] = acc

        with jax.named_scope('PRO0'):
            pro(0, True)

        def pro_rest(t, carry):
            pro(t, False)
            return carry
        with jax.named_scope('PRO1'):
            lax.fori_loop(1, D, pro_rest, 0)
        with jax.named_scope('FFN0'):
            cp_wg.wait()
            cp_wu.wait()
            cp_wd.wait()
            r0 = x1_s[0]
            f0 = _ln(r0).astype(BF16)
            acts0 = []
            FC = 512
            for c0 in range(0, FF, FC):
                wgv = pltpu.bitcast(wg_st[:, c0:c0 + FC], U32)
                wuv = pltpu.bitcast(wu_st[:, c0:c0 + FC], U32)
                wg_s[:, c0:c0 + FC] = wgv
                wu_s[:, c0:c0 + FC] = wuv
                gg = _dot(f0, _unpack(wgv))
                uu = _dot(f0, _unpack(wuv))
                acts0.append(_glu(gg, uu).astype(BF16))
            x2 = r0
            for i, c0 in enumerate(range(0, FF, FC)):
                wdv = pltpu.bitcast(wd_st[c0:c0 + FC, :], U32)
                wd_s[c0 // 2:(c0 + FC) // 2, :] = wdv
                x2 = x2 + _dot(acts0[i], _unpack(wdv))
            x2_s[0] = x2
            htok_s[1] = _pack(_ln(x2))
            cp_xr.wait()

        mask2 = make_mask(MP + 2 * SEG, [0, 1])

        def step(t, carry, ringed):
            wait_y(t - D - 1)
            x1 = x0seg(t - 1) + acc_s[MP:MP + SEG, :]
            x3 = x2_s[(t - D - 1) % XR2] + acc_s[MP + SEG:, :]
            if ringed:
                get = qkv_ring(jnp.concatenate([mem_pair(t), _unpack(htok_s[1])], axis=0), t, None)
                first = t == D
                res = jnp.concatenate([jnp.where(first, x1_s[1], x1), jnp.where(first, x1, x3)], axis=0)
                aseg = jnp.where(first, 1, t - 1)
            else:
                get = qkv_plain(jnp.concatenate([mem_pair(t), _unpack(htok_s[0]), _unpack(htok_s[1])], axis=0))
                res = jnp.concatenate([x1, x3], axis=0)
                aseg = t - 1
            fin = _ln(res).astype(BF16)
            tok1 = _ln(x0seg(t + 1))
            acts = []
            fo = []
            fillers = [lambda: acts.append(ffn_a(fin, 0, FF // 2)),
                       lambda: acts.append(ffn_a(fin, FF // 2, FF)),
                       lambda: fo.append(ffn_b(jnp.concatenate(acts, axis=1)))]
            acc = attention(get, mask2, fillers)
            xo = res + fo[0]
            acc_s[...] = acc
            x2_s[aseg % XR2] = xo[:SEG]
            if ringed:
                x2_s[jnp.where(first, 2, XR2)] = xo[SEG:]
                tok2 = _ln(jnp.where(first, xo[:SEG], x2_s[(t + 1 - D) % XR2]))
            else:
                tok2 = _ln(x2_s[(t + 1 - D) % XR2])
            htok_s[0] = _pack(tok1)
            htok_s[1] = _pack(tok2)
            emit_y(t - D - 1, xo[SEG:])
            return carry
        with jax.named_scope('PDUAL'):
            lax.fori_loop(D, D + NP, functools.partial(step, ringed=True), 0)
        with jax.named_scope('MAIN'):
            lax.fori_loop(D + NP, NSEG, functools.partial(step, ringed=False), 0)

        mask3 = make_mask(MP + SEG, [1])

        def epi(t, carry):
            wait_y(t - D - 1)
            fres_s[0] = x0seg(t - 1) + acc_s[MP:MP + SEG, :]
            fres_s[1] = x2_s[(t - D - 1) % XR2] + acc_s[MP + SEG:, :]

            @pl.when(t < NSEG + D)
            def _():
                hh = jnp.concatenate([mem_pair(t, l1_live=False), _unpack(htok_s[1])], axis=0)
                res = fres_s[1]
                fin = _ln(res).astype(BF16)
                acts = []
                fo = []
                fillers = [lambda: acts.append(ffn_a(fin, 0, FF // 2)),
                           lambda: acts.append(ffn_a(fin, FF // 2, FF)),
                           lambda: fo.append(ffn_b(jnp.concatenate(acts, axis=1)))]
                acc = attention(qkv_plain(hh), mask3, fillers)
                acc_s[:MP, :] = acc[:MP]
                acc_s[MP + SEG:, :] = acc[MP:]
                emit_y(t - D - 1, res + fo[0])

            @pl.when((t == NSEG) | (t == NSEG + D))
            def _():
                xo = ffn32(fres_s[jnp.where(t == NSEG, 0, 1)])

                @pl.when(t == NSEG)
                def _():
                    x2_s[(NSEG - 1) % XR2] = xo

                @pl.when(t == NSEG + D)
                def _():
                    emit_y(t - D - 1, xo)
            htok_s[1] = _pack(_ln(x2_s[(t + 1 - D) % XR2]))
            return carry
        with jax.named_scope('EPI'):
            lax.fori_loop(NSEG, NSEG + D + 1, epi, 0)
        out_copy(NSEG - 2, 0).wait()
        out_copy(NSEG - 1, 1).wait()

    def run(A_x, A_mem0, A_Wq, A_Wk, A_Wv, A_Wo, A_seg_len, B_x, B_w_gate, B_w_up, B_w_down):
        any_spec = pl.BlockSpec(memory_space=pl.ANY)
        out = pl.pallas_call(
            kernel,
            out_shape=jax.ShapeDtypeStruct((S, DM), BF16),
            in_specs=[any_spec] * 9,
            out_specs=any_spec,
            scratch_shapes=[
                pltpu.VMEM((NG, DM // 2, GW), U32),
                pltpu.VMEM((NG, DM // 2, GW), U32),
                pltpu.VMEM((NG, DM // 2, GW), U32),
                pltpu.VMEM((H * DH // 2, DM), U32),
                pltpu.VMEM((DM // 2, FF), U32),
                pltpu.VMEM((DM // 2, FF), U32),
                pltpu.VMEM((FF // 2, DM), U32),
                pltpu.VMEM((2, 3, DM, 8, DH), BF16),
                pltpu.VMEM((H * DH, DM), BF16),
                pltpu.VMEM((DM, FF), BF16),
                pltpu.VMEM((DM, FF), BF16),
                pltpu.VMEM((FF, DM), BF16),
                pltpu.VMEM((S, DM), BF16),
                pltpu.VMEM((M, DM), BF16),
                pltpu.VMEM((NP * SEG // 2, DM), U32),
                pltpu.VMEM((R, NG, 3, SEG // 2, GW), U32),
                pltpu.VMEM((2, SEG // 2, DM), U32),
                pltpu.VMEM((MP + 2 * SEG, DM), F32),
                pltpu.VMEM((2, SEG, DM), F32),
                pltpu.VMEM((XR2 + 1, SEG, DM), F32),
                pltpu.VMEM((2, SEG, DM), F32),
                pltpu.VMEM((2, SEG, DM), BF16),
                pltpu.SemaphoreType.DMA((2, 3)),
                pltpu.SemaphoreType.DMA((7 + WOC,)),
                pltpu.SemaphoreType.DMA((2,)),
            ],
            compiler_params=pltpu.CompilerParams(vmem_limit_bytes=124 * 1024 * 1024, disable_bounds_checks=bool(NOBC)),
            name="memtr",
        )(A_x.reshape(S, DM), A_mem0.reshape(M, DM), A_Wq, A_Wk, A_Wv, A_Wo.reshape(H * DH, DM),
          B_w_gate, B_w_up, B_w_down)
        return out.reshape(1, S, DM)
    return run


_run = _make()


@functools.partial(jax.jit, static_argnames=("A_seg_len",))
def pallas_interleave_layers__memory_aug_recurrent_mem_tr__glu_gated_glu__prompt_kernel(
    A_x, A_mem0, A_Wq, A_Wk, A_Wv, A_Wo, A_seg_len, B_x, B_w_gate, B_w_up, B_w_down,
):
    assert A_seg_len == SEG
    assert A_x.shape == (1, S, DM) and A_mem0.shape == (1, M, DM)
    assert A_Wq.shape == (DM, H, DH) and A_Wo.shape == (H, DH, DM)
    assert B_w_gate.shape == (DM, FF) and B_w_down.shape == (FF, DM)
    return _run(A_x, A_mem0, A_Wq, A_Wk, A_Wv, A_Wo, A_seg_len, B_x, B_w_gate, B_w_up, B_w_down)
```

```python
import functools
import jax
import jax.numpy as jnp
from jax import lax
from jax.experimental import pallas as pl
from jax.experimental.pallas import tpu as pltpu

S, DM, H, DH, M, SEG, FF = 2048, 1024, 32, 128, 8, 32, 3584
NSEG = S // SEG
MP = 2 * M
U32 = jnp.uint32
BF16 = jnp.bfloat16
F32 = jnp.float32
EPS = 1e-5
NEG = -1e9
LOG2E = 1.4426950408889634


def _pack(x):
    return pltpu.bitcast(x.astype(BF16), U32)


def _unpack(x):
    return pltpu.bitcast(x, BF16)


def _ln(x):
    m = jnp.mean(x, axis=-1, keepdims=True)
    xc = x - m
    v = jnp.mean(xc * xc, axis=-1, keepdims=True)
    return xc * lax.rsqrt(v + EPS)


def _glu(g, u):
    return u * pl.reciprocal(1.0 + jnp.exp2(g * (-LOG2E)), approx=True)


def _dot(a, b):
    return jnp.dot(a, b, preferred_element_type=F32)


def _make(D=3, NP=11):
    NG = 8
    HG = H // NG
    GW = HG * DH
    NOCT = H // 8
    WOC = 4
    R = NP + D
    XR2 = 4
    assert D == 3
    XH = NP + D + 1

    def kernel(x_hbm, mem0_hbm, wq_hbm, wk_hbm, wv_hbm, wo_hbm, wg_hbm, wu_hbm, wd_hbm,
               y_hbm,
               wq_s, wk_s, wv_s, wo_s, wg_s, wu_s, wd_s, st3_s, wo_st, wg_st, wu_st, wd_st,
               x0_s, mem0_ref, ptok_s, ring_s, htok_s, acc_s, x1_s, x2_s, fres_s, y_s, sem3, semw, osem):
        srcs = [wq_hbm, wk_hbm, wv_hbm]
        w3_s = [wq_s, wk_s, wv_s]

        def cp3(o, m):
            return pltpu.make_async_copy(srcs[m].at[:, pl.ds(pl.multiple_of(o * 8, 8), 8), :],
                                         st3_s.at[o % 2, m], sem3.at[o % 2, m])
        XR = XH * SEG
        XA = NP * SEG
        cp_xh = pltpu.make_async_copy(x_hbm.at[pl.ds(0, XA)], x0_s.at[pl.ds(0, XA)], semw.at[0])
        cp_xb = pltpu.make_async_copy(x_hbm.at[pl.ds(XA, XR - XA)], x0_s.at[pl.ds(XA, XR - XA)], semw.at[6 + WOC])
        cp_xr = pltpu.make_async_copy(x_hbm.at[pl.ds(XR, S - XR)], x0_s.at[pl.ds(XR, S - XR)], semw.at[1])
        cp_m0 = pltpu.make_async_copy(mem0_hbm, mem0_ref, semw.at[5 + WOC])
        WOR = H * DH // WOC
        cp_wo = [pltpu.make_async_copy(wo_hbm.at[pl.ds(c * WOR, WOR)], wo_st.at[pl.ds(c * WOR, WOR)], semw.at[2 + c])
                 for c in range(WOC)]
        cp_wg = pltpu.make_async_copy(wg_hbm, wg_st, semw.at[2 + WOC])
        cp_wu = pltpu.make_async_copy(wu_hbm, wu_st, semw.at[3 + WOC])
        cp_wd = pltpu.make_async_copy(wd_hbm, wd_st, semw.at[4 + WOC])

        def issue(descs):
            def body(i, c):
                for k, d in enumerate(descs):
                    pl.when(i == k)(d.start)
                return c
            lax.fori_loop(0, len(descs), body, 0)

        def x0seg(i):
            i = jnp.clip(i, 0, NSEG - 1)
            return x0_s[pl.ds(pl.multiple_of(i * SEG, SEG), SEG), :].astype(F32)

        sub8 = lax.broadcasted_iota(jnp.int32, (8, DH), 0)

        def conv_block(o, m, b):
            s32 = pltpu.bitcast(st3_s[o % 2, m, pl.ds(b * 16, 16)], U32).reshape(8, 2, 4, DH)
            sides = []
            for par in range(2):
                P = [jnp.concatenate([s32[k, par], s32[k + 4, par]], axis=0) for k in range(4)]
                for dist in (1, 2):
                    msk = (sub8 & dist) == 0
                    Q = list(P)
                    for k in range(4):
                        if k & dist == 0:
                            Q[k] = jnp.where(msk, P[k], pltpu.roll(P[k + dist], dist, 0))
                            Q[k + dist] = jnp.where(msk, pltpu.roll(P[k], 8 - dist, 0), P[k + dist])
                    P = Q
                sides.append(P)
            out = []
            for hp in range(4):
                out.append((sides[0][hp] & U32(0xFFFF)) | (sides[1][hp] << 16))
                out.append((sides[0][hp] >> 16) | (sides[1][hp] & U32(0xFFFF0000)))
            return out

        def pstage_m(o, m):
            p = _unpack(ptok_s[...])
            acc = None
            for k in range(DM // DH):
                blocks = [conv_block(o, m, 8 * k + b) for b in range(8)]
                w = jnp.concatenate([jnp.concatenate([blocks[b][h] for b in range(8)], axis=0)
                                     for h in range(8)], axis=1)
                for i in range(2):
                    w3_s[m][2 * o + i, pl.ds(k * 64, 64), :] = w[:, i * GW:(i + 1) * GW]
                r = _dot(p[:, k * DH:(k + 1) * DH], _unpack(w))
                acc = r if acc is None else acc + r
            r = _pack(acc)
            for i in range(2):
                for sg in range(NP):
                    ring_s[sg, 2 * o + i, m] = r[sg * 16:(sg + 1) * 16, i * GW:(i + 1) * GW]

        with jax.named_scope('P'):
            issue([cp_xh, cp3(0, 0), cp3(0, 1), cp_xb, cp_m0] + [cp3(o, m) for o in range(2) for m in range(3) if 3 * o + m > 1])
            cp_xh.wait()
            for sg in range(NP):
                ptok_s[pl.ds(sg * 16, 16), :] = _pack(_ln(x0seg(sg)))

            def pstage(o, carry):
                @pl.when(o + 2 == NOCT)
                def _():
                    issue(cp_wo + [cp_wg, cp_wu, cp_wd, cp_xr])
                for m in range(3):
                    cp3(o, m).wait()
                    pstage_m(o, m)

                    @pl.when(o + 2 < NOCT)
                    def _():
                        cp3(o + 2, m).start()
                return carry
            lax.fori_loop(0, NOCT, pstage, 0)

        c1 = (DH ** -0.5) * LOG2E

        def make_mask(rows, tok_layers):
            row = lax.broadcasted_iota(jnp.int32, (rows, rows), 0)
            col = lax.broadcasted_iota(jnp.int32, (rows, rows), 1)

            def layer(i):
                lay = jnp.where(i < M, 0, 1)
                for b, l in enumerate(tok_layers):
                    lay = jnp.where(i >= MP + b * SEG, l, lay)
                return lay
            same = layer(row) == layer(col)
            allowed = same & ((row < MP) | (col < MP) | (row >= col))
            return allowed, jnp.where(same, NEG * DH ** 0.5, -jnp.inf).astype(F32)

        def split(r):
            return [r[:, j * DH:(j + 1) * DH] for j in range(HG)]

        def qkv_plain(hh):
            def get(g):
                return [[x.astype(BF16) for x in split(_dot(hh, _unpack(w3_s[m][g])))] for m in range(3)]
            return get

        def qkv_ring(hh, rd, wr):
            def get(g):
                out = []
                for m in range(3):
                    r = _dot(hh, _unpack(w3_s[m][g]))
                    old = split(_unpack(ring_s[rd, g, m]))
                    rs = split(r)
                    if wr is None:
                        out.append([jnp.concatenate([rs[j][:MP].astype(BF16), old[j], rs[j][MP:].astype(BF16)], axis=0)
                                    for j in range(HG)])
                    else:
                        ring_s[wr, g, m] = _pack(r[MP:])
                        out.append([jnp.concatenate([rs[j][:MP].astype(BF16), old[j]], axis=0) for j in range(HG)])
                return out
            return get

        def scores(q, k):
            return [lax.dot_general(q[j], k[j], (((1,), (1,)), ((), ())), preferred_element_type=F32)
                    for j in range(HG)]

        def softmax_pv(ss, v, mask):
            os_ = []
            for j in range(HG):
                s = jnp.where(mask[0], ss[j], mask[1])
                mx = jnp.max(s, axis=-1, keepdims=True)
                e = jnp.exp2((s - mx) * c1)
                l = jnp.sum(e, axis=-1, keepdims=True)
                p = (e * pl.reciprocal(l, approx=True)).astype(BF16)
                os_.append(_dot(p, v[j]))
            return jnp.concatenate(os_, axis=1).astype(BF16)

        def wo(o, g, acc):
            r = _dot(o, _unpack(wo_s[pl.ds(g * (GW // 2), GW // 2), :]))
            return r if acc is None else acc + r

        def ffn_a(f, c0, c1_):
            gg = _dot(f, _unpack(wg_s[:, c0:c1_]))
            uu = _dot(f, _unpack(wu_s[:, c0:c1_]))
            return _glu(gg, uu).astype(BF16)

        def ffn_b(a):
            return _dot(a, _unpack(wd_s[...]))

        def ffn32(r):
            return r + ffn_b(ffn_a(_ln(r).astype(BF16), 0, FF))

        def attention(get, mask, fillers, wo=wo):
            qs, ss, oo = {}, {}, {}
            acc = None
            for i in range(NG + 3):
                if i < NG:
                    qs[i] = get(i)
                elif i - NG < len(fillers):
                    fillers[i - NG]()
                if 0 <= i - 2 < NG:
                    oo[i - 2] = softmax_pv(ss.pop(i - 2), qs.pop(i - 2)[2], mask)
                if 0 <= i - 1 < NG:
                    ss[i - 1] = scores(qs[i - 1][0], qs[i - 1][1])
                if 0 <= i - 3 < NG:
                    acc = wo(oo.pop(i - 3), i - 3, acc)
            return acc

        def out_copy(seg, slot):
            return pltpu.make_async_copy(y_s.at[slot], y_hbm.at[pl.ds(seg * SEG, SEG)], osem.at[slot])

        def wait_y(yseg):
            @pl.when(yseg >= 2)
            def _():
                out_copy(yseg - 2, yseg % 2).wait()

        def emit_y(yseg, yv):
            yslot = yseg % 2
            y_s[yslot] = yv.astype(BF16)

            @pl.when(yseg >= 0)
            def _():
                out_copy(yseg, yslot).start()

        def mem_pair(t, l1_live=True):
            mem0 = mem0_ref[...].astype(F32)
            mem1 = acc_s[:M, :] if l1_live else jnp.zeros((M, DM), F32)
            mem2 = jnp.where(t <= D, mem0, acc_s[M:MP, :])
            return jnp.concatenate([mem1, mem2], axis=0).astype(BF16)

        cp_m0.wait()
        cp_xb.wait()
        mem0 = mem0_ref[...].astype(F32)
        acc_s[...] = jnp.concatenate([mem0, mem0, jnp.zeros((2 * SEG, DM), F32)], axis=0)
        x2_s[XR2 - 1] = jnp.zeros((SEG, DM), F32)

        mask1 = make_mask(MP + SEG, [0])

        def pro(t, first):
            if not first:
                x1_s[t - 1] = x0seg(t - 1) + acc_s[MP:MP + SEG, :]
            hm = jnp.concatenate([acc_s[:M, :], mem0_ref[...].astype(F32)], axis=0).astype(BF16)
            hh = jnp.concatenate([hm, _ln(x0seg(t + NP)).astype(BF16)], axis=0)
            if first:
                for c in cp_wo:
                    c.wait()

                def wo_first(o, g, acc):
                    wov = pltpu.bitcast(wo_st[pl.ds(g * GW, GW), :], U32)
                    wo_s[pl.ds(g * (GW // 2), GW // 2), :] = wov
                    r = _dot(o, _unpack(wov))
                    return r if acc is None else acc + r
            acc = attention(qkv_ring(hh, t, t + NP), mask1, [], wo=wo_first if first else wo)
            acc_s[:MP + SEG, :] = acc

        with jax.named_scope('PRO0'):
            pro(0, True)

        def pro_rest(t, carry):
            pro(t, False)
            return carry
        with jax.named_scope('PRO1'):
            lax.fori_loop(1, D, pro_rest, 0)
        with jax.named_scope('FFN0'):
            cp_wg.wait()
            cp_wu.wait()
            cp_wd.wait()
            r0 = x1_s[0]
            f0 = _ln(r0).astype(BF16)
            acts0 = []
            FC = 512
            for c0 in range(0, FF, FC):
                wgv = pltpu.bitcast(wg_st[:, c0:c0 + FC], U32)
                wuv = pltpu.bitcast(wu_st[:, c0:c0 + FC], U32)
                wg_s[:, c0:c0 + FC] = wgv
                wu_s[:, c0:c0 + FC] = wuv
                gg = _dot(f0, _unpack(wgv))
                uu = _dot(f0, _unpack(wuv))
                acts0.append(_glu(gg, uu).astype(BF16))
            x2 = r0
            for i, c0 in enumerate(range(0, FF, FC)):
                wdv = pltpu.bitcast(wd_st[c0:c0 + FC, :], U32)
                wd_s[c0 // 2:(c0 + FC) // 2, :] = wdv
                x2 = x2 + _dot(acts0[i], _unpack(wdv))
            x2_s[0] = x2
            htok_s[1] = _pack(_ln(x2))
            cp_xr.wait()

        mask2 = make_mask(MP + 2 * SEG, [0, 1])

        def step(t, carry, ringed):
            wait_y(t - D - 1)
            x1 = x0seg(t - 1) + acc_s[MP:MP + SEG, :]
            x3 = x2_s[(t - D - 1) % XR2] + acc_s[MP + SEG:, :]
            if ringed:
                get = qkv_ring(jnp.concatenate([mem_pair(t), _unpack(htok_s[1])], axis=0), t, None)
                first = t == D
                res = jnp.concatenate([jnp.where(first, x1_s[1], x1), jnp.where(first, x1, x3)], axis=0)
                aseg = jnp.where(first, 1, t - 1)
            else:
                get = qkv_plain(jnp.concatenate([mem_pair(t), _unpack(htok_s[0]), _unpack(htok_s[1])], axis=0))
                res = jnp.concatenate([x1, x3], axis=0)
                aseg = t - 1
            fin = _ln(res).astype(BF16)
            tok1 = _ln(x0seg(t + 1))
            acts = []
            fo = []
            fillers = [lambda: acts.append(ffn_a(fin, 0, FF // 2)),
                       lambda: acts.append(ffn_a(fin, FF // 2, FF)),
                       lambda: fo.append(ffn_b(jnp.concatenate(acts, axis=1)))]
            acc = attention(get, mask2, fillers)
            xo = res + fo[0]
            acc_s[...] = acc
            x2_s[aseg % XR2] = xo[:SEG]
            if ringed:
                x2_s[jnp.where(first, 2, XR2)] = xo[SEG:]
                tok2 = _ln(jnp.where(first, xo[:SEG], x2_s[(t + 1 - D) % XR2]))
            else:
                tok2 = _ln(x2_s[(t + 1 - D) % XR2])
            htok_s[0] = _pack(tok1)
            htok_s[1] = _pack(tok2)
            emit_y(t - D - 1, xo[SEG:])
            return carry
        with jax.named_scope('PDUAL'):
            lax.fori_loop(D, D + NP, functools.partial(step, ringed=True), 0)
        with jax.named_scope('MAIN'):
            lax.fori_loop(D + NP, NSEG, functools.partial(step, ringed=False), 0)

        mask3 = make_mask(MP + SEG, [1])

        def epi(t, carry):
            wait_y(t - D - 1)
            fres_s[0] = x0seg(t - 1) + acc_s[MP:MP + SEG, :]
            fres_s[1] = x2_s[(t - D - 1) % XR2] + acc_s[MP + SEG:, :]

            @pl.when(t < NSEG + D)
            def _():
                hh = jnp.concatenate([mem_pair(t, l1_live=False), _unpack(htok_s[1])], axis=0)
                res = fres_s[1]
                fin = _ln(res).astype(BF16)
                acts = []
                fo = []
                fillers = [lambda: acts.append(ffn_a(fin, 0, FF // 2)),
                           lambda: acts.append(ffn_a(fin, FF // 2, FF)),
                           lambda: fo.append(ffn_b(jnp.concatenate(acts, axis=1)))]
                acc = attention(qkv_plain(hh), mask3, fillers)
                acc_s[:MP, :] = acc[:MP]
                acc_s[MP + SEG:, :] = acc[MP:]
                emit_y(t - D - 1, res + fo[0])

            @pl.when((t == NSEG) | (t == NSEG + D))
            def _():
                xo = ffn32(fres_s[jnp.where(t == NSEG, 0, 1)])

                @pl.when(t == NSEG)
                def _():
                    x2_s[(NSEG - 1) % XR2] = xo

                @pl.when(t == NSEG + D)
                def _():
                    emit_y(t - D - 1, xo)
            htok_s[1] = _pack(_ln(x2_s[(t + 1 - D) % XR2]))
            return carry
        with jax.named_scope('EPI'):
            lax.fori_loop(NSEG, NSEG + D + 1, epi, 0)
        out_copy(NSEG - 2, 0).wait()
        out_copy(NSEG - 1, 1).wait()

    def run(A_x, A_mem0, A_Wq, A_Wk, A_Wv, A_Wo, A_seg_len, B_x, B_w_gate, B_w_up, B_w_down):
        any_spec = pl.BlockSpec(memory_space=pl.ANY)
        out = pl.pallas_call(
            kernel,
            out_shape=jax.ShapeDtypeStruct((S, DM), BF16),
            in_specs=[any_spec] * 9,
            out_specs=any_spec,
            scratch_shapes=[
                pltpu.VMEM((NG, DM // 2, GW), U32),
                pltpu.VMEM((NG, DM // 2, GW), U32),
                pltpu.VMEM((NG, DM // 2, GW), U32),
                pltpu.VMEM((H * DH // 2, DM), U32),
                pltpu.VMEM((DM // 2, FF), U32),
                pltpu.VMEM((DM // 2, FF), U32),
                pltpu.VMEM((FF // 2, DM), U32),
                pltpu.VMEM((2, 3, DM, 8, DH), BF16),
                pltpu.VMEM((H * DH, DM), BF16),
                pltpu.VMEM((DM, FF), BF16),
                pltpu.VMEM((DM, FF), BF16),
                pltpu.VMEM((FF, DM), BF16),
                pltpu.VMEM((S, DM), BF16),
                pltpu.VMEM((M, DM), BF16),
                pltpu.VMEM((NP * SEG // 2, DM), U32),
                pltpu.VMEM((R, NG, 3, SEG // 2, GW), U32),
                pltpu.VMEM((2, SEG // 2, DM), U32),
                pltpu.VMEM((MP + 2 * SEG, DM), F32),
                pltpu.VMEM((2, SEG, DM), F32),
                pltpu.VMEM((XR2 + 1, SEG, DM), F32),
                pltpu.VMEM((2, SEG, DM), F32),
                pltpu.VMEM((2, SEG, DM), BF16),
                pltpu.SemaphoreType.DMA((2, 3)),
                pltpu.SemaphoreType.DMA((7 + WOC,)),
                pltpu.SemaphoreType.DMA((2,)),
            ],
            compiler_params=pltpu.CompilerParams(vmem_limit_bytes=124 * 1024 * 1024),
            name="memtr",
        )(A_x.reshape(S, DM), A_mem0.reshape(M, DM), A_Wq, A_Wk, A_Wv, A_Wo.reshape(H * DH, DM),
          B_w_gate, B_w_up, B_w_down)
        return out.reshape(1, S, DM)
    return run


_run = _make()


@functools.partial(jax.jit, static_argnames=("A_seg_len",))
def pallas_interleave_layers__memory_aug_recurrent_mem_tr__glu_gated_glu__prompt_kernel(
    A_x, A_mem0, A_Wq, A_Wk, A_Wv, A_Wo, A_seg_len, B_x, B_w_gate, B_w_up, B_w_down,
):
    assert A_seg_len == SEG
    assert A_x.shape == (1, S, DM) and A_mem0.shape == (1, M, DM)
    assert A_Wq.shape == (DM, H, DH) and A_Wo.shape == (H, DH, DM)
    assert B_w_gate.shape == (DM, FF) and B_w_down.shape == (FF, DM)
    return _run(A_x, A_mem0, A_Wq, A_Wk, A_Wv, A_Wo, A_seg_len, B_x, B_w_gate, B_w_up, B_w_down)
```

```python
import functools
import jax
import jax.numpy as jnp
from jax import lax
from jax.experimental import pallas as pl
from jax.experimental.pallas import tpu as pltpu

S, DM, H, DH, M, SEG, FF = 2048, 1024, 32, 128, 8, 32, 3584
NSEG = S // SEG
MP = 2 * M
U32 = jnp.uint32
BF16 = jnp.bfloat16
F32 = jnp.float32
EPS = 1e-5
NEG = -1e9
LOG2E = 1.4426950408889634


def _pack(x):
    return pltpu.bitcast(x.astype(BF16), U32)


def _unpack(x):
    return pltpu.bitcast(x, BF16)


def _ln(x):
    m = jnp.mean(x, axis=-1, keepdims=True)
    xc = x - m
    v = jnp.mean(xc * xc, axis=-1, keepdims=True)
    return xc * lax.rsqrt(v + EPS)


def _glu(g, u):
    return u * pl.reciprocal(1.0 + jnp.exp2(g * (-LOG2E)), approx=True)


def _dot(a, b):
    return jnp.dot(a, b, preferred_element_type=F32)


def _make(D=3, NP=11):
    NG = 8
    HG = H // NG
    GW = HG * DH
    NOCT = H // 8
    WOC = 4
    R = NP + D
    XR2 = 4
    assert D == 3
    XH = NP + D + 1

    def kernel(x_hbm, mem0_hbm, wq_hbm, wk_hbm, wv_hbm, wo_hbm, wg_hbm, wu_hbm, wd_hbm,
               y_hbm,
               wq_s, wk_s, wv_s, wo_s, wg_s, wu_s, wd_s, st3_s, wo_st, wg_st, wu_st, wd_st,
               x0_s, mem0_ref, ptok_s, ring_s, htok_s, acc_s, x1_s, x2_s, fres_s, y_s, sem3, semw, osem):
        srcs = [wq_hbm, wk_hbm, wv_hbm]
        w3_s = [wq_s, wk_s, wv_s]

        def cp3(o, m):
            return pltpu.make_async_copy(srcs[m].at[:, pl.ds(pl.multiple_of(o * 8, 8), 8), :],
                                         st3_s.at[o % 2, m], sem3.at[o % 2, m])
        XR = XH * SEG
        XA = NP * SEG
        cp_xh = pltpu.make_async_copy(x_hbm.at[pl.ds(0, XA)], x0_s.at[pl.ds(0, XA)], semw.at[0])
        cp_xb = pltpu.make_async_copy(x_hbm.at[pl.ds(XA, XR - XA)], x0_s.at[pl.ds(XA, XR - XA)], semw.at[6 + WOC])
        cp_xr = pltpu.make_async_copy(x_hbm.at[pl.ds(XR, S - XR)], x0_s.at[pl.ds(XR, S - XR)], semw.at[1])
        cp_m0 = pltpu.make_async_copy(mem0_hbm, mem0_ref, semw.at[5 + WOC])
        WOR = H * DH // WOC
        cp_wo = [pltpu.make_async_copy(wo_hbm.at[pl.ds(c * WOR, WOR)], wo_st.at[pl.ds(c * WOR, WOR)], semw.at[2 + c])
                 for c in range(WOC)]
        cp_wg = pltpu.make_async_copy(wg_hbm, wg_st, semw.at[2 + WOC])
        cp_wu = pltpu.make_async_copy(wu_hbm, wu_st, semw.at[3 + WOC])
        cp_wd = pltpu.make_async_copy(wd_hbm, wd_st, semw.at[4 + WOC])

        def issue(descs):
            def body(i, c):
                for k, d in enumerate(descs):
                    pl.when(i == k)(d.start)
                return c
            lax.fori_loop(0, len(descs), body, 0)

        def x0seg(i):
            i = jnp.clip(i, 0, NSEG - 1)
            return x0_s[pl.ds(pl.multiple_of(i * SEG, SEG), SEG), :].astype(F32)

        sub8 = lax.broadcasted_iota(jnp.int32, (8, DH), 0)

        def conv_block(o, m, b):
            s32 = pltpu.bitcast(st3_s[o % 2, m, pl.ds(b * 16, 16)], U32).reshape(8, 2, 4, DH)
            sides = []
            for par in range(2):
                P = [jnp.concatenate([s32[k, par], s32[k + 4, par]], axis=0) for k in range(4)]
                for dist in (1, 2):
                    msk = (sub8 & dist) == 0
                    Q = list(P)
                    for k in range(4):
                        if k & dist == 0:
                            Q[k] = jnp.where(msk, P[k], pltpu.roll(P[k + dist], dist, 0))
                            Q[k + dist] = jnp.where(msk, pltpu.roll(P[k], 8 - dist, 0), P[k + dist])
                    P = Q
                sides.append(P)
            out = []
            for hp in range(4):
                out.append((sides[0][hp] & U32(0xFFFF)) | (sides[1][hp] << 16))
                out.append((sides[0][hp] >> 16) | (sides[1][hp] & U32(0xFFFF0000)))
            return out

        def pstage_m(o, m):
            p = _unpack(ptok_s[...])
            acc = None
            for k in range(DM // DH):
                blocks = [conv_block(o, m, 8 * k + b) for b in range(8)]
                w = jnp.concatenate([jnp.concatenate([blocks[b][h] for b in range(8)], axis=0)
                                     for h in range(8)], axis=1)
                for i in range(2):
                    w3_s[m][2 * o + i, pl.ds(k * 64, 64), :] = w[:, i * GW:(i + 1) * GW]
                r = _dot(p[:, k * DH:(k + 1) * DH], _unpack(w))
                acc = r if acc is None else acc + r
            r = _pack(acc)
            for i in range(2):
                for sg in range(NP):
                    ring_s[sg, 2 * o + i, m] = r[sg * 16:(sg + 1) * 16, i * GW:(i + 1) * GW]

        with jax.named_scope('P'):
            issue([cp_xh, cp3(0, 0), cp3(0, 1), cp_xb, cp_m0] + [cp3(o, m) for o in range(2) for m in range(3) if 3 * o + m > 1])
            cp_xh.wait()
            for sg in range(NP):
                ptok_s[pl.ds(sg * 16, 16), :] = _pack(_ln(x0seg(sg)))

            def pstage(o, carry):
                @pl.when(o + 2 == NOCT)
                def _():
                    issue(cp_wo + [cp_wg, cp_wu, cp_wd, cp_xr])
                for m in range(3):
                    cp3(o, m).wait()
                    pstage_m(o, m)

                    @pl.when(o + 2 < NOCT)
                    def _():
                        cp3(o + 2, m).start()
                return carry
            lax.fori_loop(0, NOCT, pstage, 0)

        c1 = (DH ** -0.5) * LOG2E

        def make_mask(rows, tok_layers):
            row = lax.broadcasted_iota(jnp.int32, (rows, rows), 0)
            col = lax.broadcasted_iota(jnp.int32, (rows, rows), 1)

            def layer(i):
                lay = jnp.where(i < M, 0, 1)
                for b, l in enumerate(tok_layers):
                    lay = jnp.where(i >= MP + b * SEG, l, lay)
                return lay
            same = layer(row) == layer(col)
            allowed = same & ((row < MP) | (col < MP) | (row >= col))
            return allowed, jnp.where(same, NEG * DH ** 0.5, -jnp.inf).astype(F32)

        def split(r):
            return [r[:, j * DH:(j + 1) * DH] for j in range(HG)]

        def qkv_plain(hh):
            def get(g):
                return [[x.astype(BF16) for x in split(_dot(hh, _unpack(w3_s[m][g])))] for m in range(3)]
            return get

        def qkv_ring(hh, rd, wr):
            def get(g):
                out = []
                for m in range(3):
                    r = _dot(hh, _unpack(w3_s[m][g]))
                    old = split(_unpack(ring_s[rd, g, m]))
                    rs = split(r)
                    if wr is None:
                        out.append([jnp.concatenate([rs[j][:MP].astype(BF16), old[j], rs[j][MP:].astype(BF16)], axis=0)
                                    for j in range(HG)])
                    else:
                        ring_s[wr, g, m] = _pack(r[MP:])
                        out.append([jnp.concatenate([rs[j][:MP].astype(BF16), old[j]], axis=0) for j in range(HG)])
                return out
            return get

        def scores(q, k):
            return [lax.dot_general(q[j], k[j], (((1,), (1,)), ((), ())), preferred_element_type=F32)
                    for j in range(HG)]

        def softmax_pv(ss, v, mask):
            os_ = []
            for j in range(HG):
                s = jnp.where(mask[0], ss[j], mask[1])
                mx = jnp.max(s, axis=-1, keepdims=True)
                e = jnp.exp2((s - mx) * c1)
                l = jnp.sum(e, axis=-1, keepdims=True)
                p = (e * pl.reciprocal(l, approx=True)).astype(BF16)
                os_.append(_dot(p, v[j]))
            return jnp.concatenate(os_, axis=1).astype(BF16)

        def wo(o, g, acc):
            r = _dot(o, _unpack(wo_s[pl.ds(g * (GW // 2), GW // 2), :]))
            return r if acc is None else acc + r

        def ffn_a(f, c0, c1_):
            gg = _dot(f, _unpack(wg_s[:, c0:c1_]))
            uu = _dot(f, _unpack(wu_s[:, c0:c1_]))
            return _glu(gg, uu).astype(BF16)

        def ffn_b(a):
            return _dot(a, _unpack(wd_s[...]))

        def ffn32(r):
            return r + ffn_b(ffn_a(_ln(r).astype(BF16), 0, FF))

        def attention(get, mask, fillers, wo=wo):
            qs, ss, oo = {}, {}, {}
            acc = None
            for i in range(NG + 3):
                if i < NG:
                    qs[i] = get(i)
                elif i - NG < len(fillers):
                    fillers[i - NG]()
                if 0 <= i - 2 < NG:
                    oo[i - 2] = softmax_pv(ss.pop(i - 2), qs.pop(i - 2)[2], mask)
                if 0 <= i - 1 < NG:
                    ss[i - 1] = scores(qs[i - 1][0], qs[i - 1][1])
                if 0 <= i - 3 < NG:
                    acc = wo(oo.pop(i - 3), i - 3, acc)
            return acc

        def out_copy(seg, slot):
            return pltpu.make_async_copy(y_s.at[slot], y_hbm.at[pl.ds(seg * SEG, SEG)], osem.at[slot])

        def wait_y(yseg):
            @pl.when(yseg >= 2)
            def _():
                out_copy(yseg - 2, yseg % 2).wait()

        def emit_y(yseg, yv):
            yslot = yseg % 2
            y_s[yslot] = yv.astype(BF16)

            @pl.when(yseg >= 0)
            def _():
                out_copy(yseg, yslot).start()

        def mem_pair(t, l1_live=True):
            mem0 = mem0_ref[...].astype(F32)
            mem1 = acc_s[:M, :] if l1_live else jnp.zeros((M, DM), F32)
            mem2 = jnp.where(t <= D, mem0, acc_s[M:MP, :])
            return jnp.concatenate([mem1, mem2], axis=0).astype(BF16)

        cp_m0.wait()
        cp_xb.wait()
        mem0 = mem0_ref[...].astype(F32)
        acc_s[...] = jnp.concatenate([mem0, mem0, jnp.zeros((2 * SEG, DM), F32)], axis=0)
        x2_s[XR2 - 1] = jnp.zeros((SEG, DM), F32)
        htok_s[0] = _pack(_ln(x0seg(NP)))

        mask1 = make_mask(MP + SEG, [0])

        def pro(t, first):
            if not first:
                x1_s[t - 1] = x0seg(t - 1) + acc_s[MP:MP + SEG, :]
            hm = jnp.concatenate([acc_s[:M, :], mem0_ref[...].astype(F32)], axis=0).astype(BF16)
            hh = jnp.concatenate([hm, _unpack(htok_s[0])], axis=0)
            nxt = _ln(x0seg(t + 1 + NP))
            if not first:
                fin0 = _ln(x1_s[0])
            if first:
                for c in cp_wo:
                    c.wait()

                def wo_first(o, g, acc):
                    wov = pltpu.bitcast(wo_st[pl.ds(g * GW, GW), :], U32)
                    wo_s[pl.ds(g * (GW // 2), GW // 2), :] = wov
                    r = _dot(o, _unpack(wov))
                    return r if acc is None else acc + r
            acc = attention(qkv_ring(hh, t, t + NP), mask1, [], wo=wo_first if first else wo)
            acc_s[:MP + SEG, :] = acc
            htok_s[0] = _pack(nxt)
            if not first:
                htok_s[1] = _pack(fin0)

        with jax.named_scope('PRO0'):
            pro(0, True)

        def pro_rest(t, carry):
            pro(t, False)
            return carry
        with jax.named_scope('PRO1'):
            lax.fori_loop(1, D, pro_rest, 0)
        with jax.named_scope('FFN0'):
            cp_wg.wait()
            cp_wu.wait()
            cp_wd.wait()
            r0 = x1_s[0]
            f0 = _unpack(htok_s[1])
            acts0 = []
            FC = 512
            for c0 in range(0, FF, FC):
                wgv = pltpu.bitcast(wg_st[:, c0:c0 + FC], U32)
                wuv = pltpu.bitcast(wu_st[:, c0:c0 + FC], U32)
                wg_s[:, c0:c0 + FC] = wgv
                wu_s[:, c0:c0 + FC] = wuv
                gg = _dot(f0, _unpack(wgv))
                uu = _dot(f0, _unpack(wuv))
                acts0.append(_glu(gg, uu).astype(BF16))
            x2 = r0
            for i, c0 in enumerate(range(0, FF, FC)):
                wdv = pltpu.bitcast(wd_st[c0:c0 + FC, :], U32)
                wd_s[c0 // 2:(c0 + FC) // 2, :] = wdv
                x2 = x2 + _dot(acts0[i], _unpack(wdv))
            x2_s[0] = x2
            htok_s[1] = _pack(_ln(x2))
            cp_xr.wait()

        mask2 = make_mask(MP + 2 * SEG, [0, 1])

        def step(t, carry, ringed):
            wait_y(t - D - 1)
            x1 = x0seg(t - 1) + acc_s[MP:MP + SEG, :]
            x3 = x2_s[(t - D - 1) % XR2] + acc_s[MP + SEG:, :]
            if ringed:
                get = qkv_ring(jnp.concatenate([mem_pair(t), _unpack(htok_s[1])], axis=0), t, None)
                first = t == D
                res = jnp.concatenate([jnp.where(first, x1_s[1], x1), jnp.where(first, x1, x3)], axis=0)
                aseg = jnp.where(first, 1, t - 1)
            else:
                get = qkv_plain(jnp.concatenate([mem_pair(t), _unpack(htok_s[0]), _unpack(htok_s[1])], axis=0))
                res = jnp.concatenate([x1, x3], axis=0)
                aseg = t - 1
            fin = _ln(res).astype(BF16)
            tok1 = _ln(x0seg(t + 1))
            acts = []
            fo = []
            fillers = [lambda: acts.append(ffn_a(fin, 0, FF // 2)),
                       lambda: acts.append(ffn_a(fin, FF // 2, FF)),
                       lambda: fo.append(ffn_b(jnp.concatenate(acts, axis=1)))]
            acc = attention(get, mask2, fillers)
            xo = res + fo[0]
            acc_s[...] = acc
            x2_s[aseg % XR2] = xo[:SEG]
            if ringed:
                x2_s[jnp.where(first, 2, XR2)] = xo[SEG:]
                tok2 = _ln(jnp.where(first, xo[:SEG], x2_s[(t + 1 - D) % XR2]))
            else:
                tok2 = _ln(x2_s[(t + 1 - D) % XR2])
            htok_s[0] = _pack(tok1)
            htok_s[1] = _pack(tok2)
            emit_y(t - D - 1, xo[SEG:])
            return carry
        with jax.named_scope('PDUAL'):
            lax.fori_loop(D, D + NP, functools.partial(step, ringed=True), 0)
        with jax.named_scope('MAIN'):
            lax.fori_loop(D + NP, NSEG, functools.partial(step, ringed=False), 0)

        mask3 = make_mask(MP + SEG, [1])

        def epi(t, carry):
            wait_y(t - D - 1)
            fres_s[0] = x0seg(t - 1) + acc_s[MP:MP + SEG, :]
            fres_s[1] = x2_s[(t - D - 1) % XR2] + acc_s[MP + SEG:, :]

            @pl.when(t < NSEG + D)
            def _():
                hh = jnp.concatenate([mem_pair(t, l1_live=False), _unpack(htok_s[1])], axis=0)
                res = fres_s[1]
                fin = _ln(res).astype(BF16)
                acts = []
                fo = []
                fillers = [lambda: acts.append(ffn_a(fin, 0, FF // 2)),
                           lambda: acts.append(ffn_a(fin, FF // 2, FF)),
                           lambda: fo.append(ffn_b(jnp.concatenate(acts, axis=1)))]
                acc = attention(qkv_plain(hh), mask3, fillers)
                acc_s[:MP, :] = acc[:MP]
                acc_s[MP + SEG:, :] = acc[MP:]
                emit_y(t - D - 1, res + fo[0])

            @pl.when((t == NSEG) | (t == NSEG + D))
            def _():
                xo = ffn32(fres_s[jnp.where(t == NSEG, 0, 1)])

                @pl.when(t == NSEG)
                def _():
                    x2_s[(NSEG - 1) % XR2] = xo

                @pl.when(t == NSEG + D)
                def _():
                    emit_y(t - D - 1, xo)
            htok_s[1] = _pack(_ln(x2_s[(t + 1 - D) % XR2]))
            return carry
        with jax.named_scope('EPI'):
            lax.fori_loop(NSEG, NSEG + D + 1, epi, 0)
        out_copy(NSEG - 2, 0).wait()
        out_copy(NSEG - 1, 1).wait()

    def run(A_x, A_mem0, A_Wq, A_Wk, A_Wv, A_Wo, A_seg_len, B_x, B_w_gate, B_w_up, B_w_down):
        any_spec = pl.BlockSpec(memory_space=pl.ANY)
        out = pl.pallas_call(
            kernel,
            out_shape=jax.ShapeDtypeStruct((S, DM), BF16),
            in_specs=[any_spec] * 9,
            out_specs=any_spec,
            scratch_shapes=[
                pltpu.VMEM((NG, DM // 2, GW), U32),
                pltpu.VMEM((NG, DM // 2, GW), U32),
                pltpu.VMEM((NG, DM // 2, GW), U32),
                pltpu.VMEM((H * DH // 2, DM), U32),
                pltpu.VMEM((DM // 2, FF), U32),
                pltpu.VMEM((DM // 2, FF), U32),
                pltpu.VMEM((FF // 2, DM), U32),
                pltpu.VMEM((2, 3, DM, 8, DH), BF16),
                pltpu.VMEM((H * DH, DM), BF16),
                pltpu.VMEM((DM, FF), BF16),
                pltpu.VMEM((DM, FF), BF16),
                pltpu.VMEM((FF, DM), BF16),
                pltpu.VMEM((S, DM), BF16),
                pltpu.VMEM((M, DM), BF16),
                pltpu.VMEM((NP * SEG // 2, DM), U32),
                pltpu.VMEM((R, NG, 3, SEG // 2, GW), U32),
                pltpu.VMEM((2, SEG // 2, DM), U32),
                pltpu.VMEM((MP + 2 * SEG, DM), F32),
                pltpu.VMEM((2, SEG, DM), F32),
                pltpu.VMEM((XR2 + 1, SEG, DM), F32),
                pltpu.VMEM((2, SEG, DM), F32),
                pltpu.VMEM((2, SEG, DM), BF16),
                pltpu.SemaphoreType.DMA((2, 3)),
                pltpu.SemaphoreType.DMA((7 + WOC,)),
                pltpu.SemaphoreType.DMA((2,)),
            ],
            compiler_params=pltpu.CompilerParams(vmem_limit_bytes=124 * 1024 * 1024),
            name="memtr",
        )(A_x.reshape(S, DM), A_mem0.reshape(M, DM), A_Wq, A_Wk, A_Wv, A_Wo.reshape(H * DH, DM),
          B_w_gate, B_w_up, B_w_down)
        return out.reshape(1, S, DM)
    return run


_run = _make()


@functools.partial(jax.jit, static_argnames=("A_seg_len",))
def pallas_interleave_layers__memory_aug_recurrent_mem_tr__glu_gated_glu__prompt_kernel(
    A_x, A_mem0, A_Wq, A_Wk, A_Wv, A_Wo, A_seg_len, B_x, B_w_gate, B_w_up, B_w_down,
):
    assert A_seg_len == SEG
    assert A_x.shape == (1, S, DM) and A_mem0.shape == (1, M, DM)
    assert A_Wq.shape == (DM, H, DH) and A_Wo.shape == (H, DH, DM)
    assert B_w_gate.shape == (DM, FF) and B_w_down.shape == (FF, DM)
    return _run(A_x, A_mem0, A_Wq, A_Wk, A_Wv, A_Wo, A_seg_len, B_x, B_w_gate, B_w_up, B_w_down)
```

```python
import functools
import jax
import jax.numpy as jnp
from jax import lax
from jax.experimental import pallas as pl
from jax.experimental.pallas import tpu as pltpu

S, DM, H, DH, M, SEG, FF = 2048, 1024, 32, 128, 8, 32, 3584
NSEG = S // SEG
MP = 2 * M
U32 = jnp.uint32
BF16 = jnp.bfloat16
F32 = jnp.float32
EPS = 1e-5
NEG = -1e9
LOG2E = 1.4426950408889634


def _pack(x):
    return pltpu.bitcast(x.astype(BF16), U32)


def _unpack(x):
    return pltpu.bitcast(x, BF16)


def _ln(x):
    m = jnp.mean(x, axis=-1, keepdims=True)
    xc = x - m
    v = jnp.mean(xc * xc, axis=-1, keepdims=True)
    return xc * lax.rsqrt(v + EPS)


def _glu(g, u):
    return u * pl.reciprocal(1.0 + jnp.exp2(g * (-LOG2E)), approx=True)


def _dot(a, b):
    return jnp.dot(a, b, preferred_element_type=F32)


def _make(D=2, NP=13):
    NG = 8
    HG = H // NG
    GW = HG * DH
    NOCT = H // 8
    WOC = 4
    R = NP + D
    XR2 = 4
    assert D == 2
    XH = NP + D + 1

    def kernel(x_hbm, mem0_hbm, wq_hbm, wk_hbm, wv_hbm, wo_hbm, wg_hbm, wu_hbm, wd_hbm,
               y_hbm,
               wq_s, wk_s, wv_s, wo_s, wg_s, wu_s, wd_s, st3_s, wo_st, wg_st, wu_st, wd_st,
               x0_s, mem0_ref, ptok_s, ring_s, htok_s, acc_s, x1_s, x2_s, fres_s, y_s, sem3, semw, osem):
        srcs = [wq_hbm, wk_hbm, wv_hbm]
        w3_s = [wq_s, wk_s, wv_s]

        def cp3(o, m):
            return pltpu.make_async_copy(srcs[m].at[:, pl.ds(pl.multiple_of(o * 8, 8), 8), :],
                                         st3_s.at[o % 2, m], sem3.at[(o % 2) * 3 + m])
        XR = XH * SEG
        XA = NP * SEG
        cp_xh = pltpu.make_async_copy(x_hbm.at[pl.ds(0, XA)], x0_s.at[pl.ds(0, XA)], semw.at[0])
        cp_xb = pltpu.make_async_copy(x_hbm.at[pl.ds(XA, XR - XA)], x0_s.at[pl.ds(XA, XR - XA)], semw.at[6 + WOC])
        cp_xr = pltpu.make_async_copy(x_hbm.at[pl.ds(XR, S - XR)], x0_s.at[pl.ds(XR, S - XR)], semw.at[1])
        cp_m0 = pltpu.make_async_copy(mem0_hbm, mem0_ref, semw.at[5 + WOC])
        WOR = H * DH // WOC
        cp_wo = [pltpu.make_async_copy(wo_hbm.at[pl.ds(c * WOR, WOR)], wo_st.at[pl.ds(c * WOR, WOR)], semw.at[2 + c])
                 for c in range(WOC)]
        cp_wg = pltpu.make_async_copy(wg_hbm, wg_st, semw.at[2 + WOC])
        cp_wu = pltpu.make_async_copy(wu_hbm, wu_st, semw.at[3 + WOC])
        cp_wd = pltpu.make_async_copy(wd_hbm, wd_st, semw.at[4 + WOC])

        def issue(descs):
            def body(i, c):
                for k, d in enumerate(descs):
                    pl.when(i == k)(d.start)
                return c
            lax.fori_loop(0, len(descs), body, 0)

        def x0seg(i):
            i = jnp.clip(i, 0, NSEG - 1)
            return x0_s[pl.ds(pl.multiple_of(i * SEG, SEG), SEG), :].astype(F32)

        sub8 = lax.broadcasted_iota(jnp.int32, (8, DH), 0)

        def conv_block(o, m, b):
            s32 = pltpu.bitcast(st3_s[o % 2, m, pl.ds(b * 16, 16)], U32).reshape(8, 2, 4, DH)
            sides = []
            for par in range(2):
                P = [jnp.concatenate([s32[k, par], s32[k + 4, par]], axis=0) for k in range(4)]
                for dist in (1, 2):
                    msk = (sub8 & dist) == 0
                    Q = list(P)
                    for k in range(4):
                        if k & dist == 0:
                            Q[k] = jnp.where(msk, P[k], pltpu.roll(P[k + dist], dist, 0))
                            Q[k + dist] = jnp.where(msk, pltpu.roll(P[k], 8 - dist, 0), P[k + dist])
                    P = Q
                sides.append(P)
            out = []
            for hp in range(4):
                out.append((sides[0][hp] & U32(0xFFFF)) | (sides[1][hp] << 16))
                out.append((sides[0][hp] >> 16) | (sides[1][hp] & U32(0xFFFF0000)))
            return out

        def pstage_m(o, m):
            p = _unpack(ptok_s[...])
            acc = None
            for k in range(DM // DH):
                blocks = [conv_block(o, m, 8 * k + b) for b in range(8)]
                w = jnp.concatenate([jnp.concatenate([blocks[b][h] for b in range(8)], axis=0)
                                     for h in range(8)], axis=1)
                for i in range(2):
                    w3_s[m][2 * o + i, pl.ds(k * 64, 64), :] = w[:, i * GW:(i + 1) * GW]
                r = _dot(p[:, k * DH:(k + 1) * DH], _unpack(w))
                acc = r if acc is None else acc + r
            r = _pack(acc)
            for i in range(2):
                for sg in range(NP):
                    ring_s[sg, 2 * o + i, m] = r[sg * 16:(sg + 1) * 16, i * GW:(i + 1) * GW]

        with jax.named_scope('P'):
            issue([cp_xh, cp3(0, 0), cp3(0, 1), cp_xb, cp_m0] + [cp3(o, m) for o in range(2) for m in range(3) if 3 * o + m > 1])
            cp_xh.wait()
            for sg in range(NP):
                ptok_s[pl.ds(sg * 16, 16), :] = _pack(_ln(x0seg(sg)))

            def pstage(o, carry):
                @pl.when(o + 2 == NOCT)
                def _():
                    issue(cp_wo + [cp_wg, cp_wu, cp_wd, cp_xr])
                for m in range(3):
                    cp3(o, m).wait()
                    pstage_m(o, m)

                    @pl.when(o + 2 < NOCT)
                    def _():
                        cp3(o + 2, m).start()
                return carry
            lax.fori_loop(0, NOCT, pstage, 0)

        c1 = (DH ** -0.5) * LOG2E

        def make_mask(rows, tok_layers):
            row = lax.broadcasted_iota(jnp.int32, (rows, rows), 0)
            col = lax.broadcasted_iota(jnp.int32, (rows, rows), 1)

            def layer(i):
                lay = jnp.where(i < M, 0, 1)
                for b, l in enumerate(tok_layers):
                    lay = jnp.where(i >= MP + b * SEG, l, lay)
                return lay
            same = layer(row) == layer(col)
            allowed = same & ((row < MP) | (col < MP) | (row >= col))
            return allowed, jnp.where(same, NEG * DH ** 0.5, -jnp.inf).astype(F32)

        def split(r):
            return [r[:, j * DH:(j + 1) * DH] for j in range(HG)]

        def qkv_plain(hh):
            def get(g):
                return [[x.astype(BF16) for x in split(_dot(hh, _unpack(w3_s[m][g])))] for m in range(3)]
            return get

        def qkv_ring(hh, rd, wr):
            def get(g):
                out = []
                for m in range(3):
                    r = _dot(hh, _unpack(w3_s[m][g]))
                    old = split(_unpack(ring_s[rd, g, m]))
                    rs = split(r)
                    if wr is None:
                        out.append([jnp.concatenate([rs[j][:MP].astype(BF16), old[j], rs[j][MP:].astype(BF16)], axis=0)
                                    for j in range(HG)])
                    else:
                        ring_s[wr, g, m] = _pack(r[MP:])
                        out.append([jnp.concatenate([rs[j][:MP].astype(BF16), old[j]], axis=0) for j in range(HG)])
                return out
            return get

        def scores(q, k):
            return [lax.dot_general(q[j], k[j], (((1,), (1,)), ((), ())), preferred_element_type=F32)
                    for j in range(HG)]

        def softmax_pv(ss, v, mask):
            os_ = []
            for j in range(HG):
                s = jnp.where(mask[0], ss[j], mask[1])
                mx = jnp.max(s, axis=-1, keepdims=True)
                e = jnp.exp2((s - mx) * c1)
                l = jnp.sum(e, axis=-1, keepdims=True)
                p = (e * pl.reciprocal(l, approx=True)).astype(BF16)
                os_.append(_dot(p, v[j]))
            return jnp.concatenate(os_, axis=1).astype(BF16)

        def wo(o, g, acc):
            r = _dot(o, _unpack(wo_s[pl.ds(g * (GW // 2), GW // 2), :]))
            return r if acc is None else acc + r

        def ffn_a(f, c0, c1_):
            gg = _dot(f, _unpack(wg_s[:, c0:c1_]))
            uu = _dot(f, _unpack(wu_s[:, c0:c1_]))
            return _glu(gg, uu).astype(BF16)

        def ffn_b(a):
            return _dot(a, _unpack(wd_s[...]))

        def ffn32(r):
            return r + ffn_b(ffn_a(_ln(r).astype(BF16), 0, FF))

        def attention(get, mask, fillers, wo=wo):
            qs, ss, oo = {}, {}, {}
            acc = None
            for i in range(NG + 3):
                if i < NG:
                    qs[i] = get(i)
                elif i - NG < len(fillers):
                    fillers[i - NG]()
                if 0 <= i - 2 < NG:
                    oo[i - 2] = softmax_pv(ss.pop(i - 2), qs.pop(i - 2)[2], mask)
                if 0 <= i - 1 < NG:
                    ss[i - 1] = scores(qs[i - 1][0], qs[i - 1][1])
                if 0 <= i - 3 < NG:
                    acc = wo(oo.pop(i - 3), i - 3, acc)
            return acc

        def out_copy(seg, slot):
            return pltpu.make_async_copy(y_s.at[slot], y_hbm.at[pl.ds(seg * SEG, SEG)], osem.at[slot])

        def wait_y(yseg):
            @pl.when(yseg >= 2)
            def _():
                out_copy(yseg - 2, yseg % 2).wait()

        def emit_y(yseg, yv):
            yslot = yseg % 2
            y_s[yslot] = yv.astype(BF16)

            @pl.when(yseg >= 0)
            def _():
                out_copy(yseg, yslot).start()

        def mem_pair(t, l1_live=True):
            mem0 = mem0_ref[...].astype(F32)
            mem1 = acc_s[:M, :] if l1_live else jnp.zeros((M, DM), F32)
            mem2 = jnp.where(t <= D, mem0, acc_s[M:MP, :])
            return jnp.concatenate([mem1, mem2], axis=0).astype(BF16)

        cp_m0.wait()
        cp_xb.wait()
        mem0 = mem0_ref[...].astype(F32)
        acc_s[...] = jnp.concatenate([mem0, mem0, jnp.zeros((2 * SEG, DM), F32)], axis=0)
        htok_s[0] = _pack(_ln(x0seg(NP)))

        mask1 = make_mask(MP + SEG, [0])

        def pro(t, carry):
            @pl.when(t == 0)
            def _():
                for c in cp_wo:
                    c.wait()
            hm = jnp.concatenate([acc_s[:M, :], mem0_ref[...].astype(F32)], axis=0).astype(BF16)
            hh = jnp.concatenate([hm, _unpack(htok_s[0])], axis=0)
            nxt = _ln(x0seg(t + 1 + NP))
            x1_s[...] = x0seg(t - 1) + acc_s[MP:MP + SEG, :]

            def wo_fn(o, g, acc):
                wov = pltpu.bitcast(wo_st[pl.ds(g * GW, GW), :], U32)
                wo_s[pl.ds(g * (GW // 2), GW // 2), :] = wov
                r = _dot(o, _unpack(wov))
                return r if acc is None else acc + r
            acc = attention(qkv_ring(hh, t, t + NP), mask1, [], wo=wo_fn)
            acc_s[:MP + SEG, :] = acc
            htok_s[0] = _pack(nxt)
            return carry

        with jax.named_scope('PRO'):
            lax.fori_loop(0, D, pro, 0)
        with jax.named_scope('FFN0'):
            cp_wg.wait()
            cp_wu.wait()
            cp_wd.wait()
            r0 = jnp.concatenate([x1_s[...], x0seg(1) + acc_s[MP:MP + SEG, :]], axis=0)
            f0 = _ln(r0).astype(BF16)
            acts0 = []
            FC = 512
            for c0 in range(0, FF, FC):
                wgv = pltpu.bitcast(wg_st[:, c0:c0 + FC], U32)
                wuv = pltpu.bitcast(wu_st[:, c0:c0 + FC], U32)
                wg_s[:, c0:c0 + FC] = wgv
                wu_s[:, c0:c0 + FC] = wuv
                gg = _dot(f0, _unpack(wgv))
                uu = _dot(f0, _unpack(wuv))
                acts0.append(_glu(gg, uu).astype(BF16))
            x2 = r0
            for i, c0 in enumerate(range(0, FF, FC)):
                wdv = pltpu.bitcast(wd_st[c0:c0 + FC, :], U32)
                wd_s[c0 // 2:(c0 + FC) // 2, :] = wdv
                x2 = x2 + _dot(acts0[i], _unpack(wdv))
            x2_s[0] = x2[:SEG]
            x2_s[1] = x2[SEG:]
            htok_s[1] = _pack(_ln(x2[:SEG]))
            cp_xr.wait()

        mask2 = make_mask(MP + 2 * SEG, [0, 1])

        def step(t, carry, ringed, glu=True):
            if glu:
                wait_y(t - D - 1)
            if ringed:
                get = qkv_ring(jnp.concatenate([mem_pair(t), _unpack(htok_s[1])], axis=0), t, None)
            else:
                get = qkv_plain(jnp.concatenate([mem_pair(t), _unpack(htok_s[0]), _unpack(htok_s[1])], axis=0))
            tok1 = _ln(x0seg(t + 1))
            fillers = []
            if glu:
                res = jnp.concatenate([x0seg(t - 1) + acc_s[MP:MP + SEG, :],
                                       x2_s[(t - D - 1) % XR2] + acc_s[MP + SEG:, :]], axis=0)
                fin = _ln(res).astype(BF16)
                acts = []
                fo = []
                fillers = [lambda: acts.append(ffn_a(fin, 0, FF // 2)),
                           lambda: acts.append(ffn_a(fin, FF // 2, FF)),
                           lambda: fo.append(ffn_b(jnp.concatenate(acts, axis=1)))]
            acc = attention(get, mask2, fillers)
            acc_s[...] = acc
            htok_s[0] = _pack(tok1)
            if glu:
                xo = res + fo[0]
                x2_s[(t - 1) % XR2] = xo[:SEG]
                htok_s[1] = _pack(_ln(xo[:SEG]))
                emit_y(t - D - 1, xo[SEG:])
            else:
                htok_s[1] = _pack(_ln(x2_s[1]))
            return carry
        with jax.named_scope('PD0'):
            step(D, 0, ringed=True, glu=False)
        with jax.named_scope('PDUAL'):
            lax.fori_loop(D + 1, D + NP, functools.partial(step, ringed=True), 0)
        with jax.named_scope('MAIN'):
            lax.fori_loop(D + NP, NSEG, functools.partial(step, ringed=False), 0)

        mask3 = make_mask(MP + SEG, [1])

        def epi(t, carry):
            wait_y(t - D - 1)
            fres_s[0] = x0seg(t - 1) + acc_s[MP:MP + SEG, :]
            fres_s[1] = x2_s[(t - D - 1) % XR2] + acc_s[MP + SEG:, :]

            @pl.when(t < NSEG + D)
            def _():
                hh = jnp.concatenate([mem_pair(t, l1_live=False), _unpack(htok_s[1])], axis=0)
                res = fres_s[1]
                fin = _ln(res).astype(BF16)
                acts = []
                fo = []
                fillers = [lambda: acts.append(ffn_a(fin, 0, FF // 2)),
                           lambda: acts.append(ffn_a(fin, FF // 2, FF)),
                           lambda: fo.append(ffn_b(jnp.concatenate(acts, axis=1)))]
                acc = attention(qkv_plain(hh), mask3, fillers)
                acc_s[:MP, :] = acc[:MP]
                acc_s[MP + SEG:, :] = acc[MP:]
                emit_y(t - D - 1, res + fo[0])

            @pl.when((t == NSEG) | (t == NSEG + D))
            def _():
                xo = ffn32(fres_s[jnp.where(t == NSEG, 0, 1)])

                @pl.when(t == NSEG)
                def _():
                    x2_s[(NSEG - 1) % XR2] = xo
                    htok_s[1] = _pack(_ln(xo))

                @pl.when(t == NSEG + D)
                def _():
                    emit_y(t - D - 1, xo)
            return carry
        with jax.named_scope('EPI'):
            lax.fori_loop(NSEG, NSEG + D + 1, epi, 0)
        out_copy(NSEG - 2, 0).wait()
        out_copy(NSEG - 1, 1).wait()

    def run(A_x, A_mem0, A_Wq, A_Wk, A_Wv, A_Wo, A_seg_len, B_x, B_w_gate, B_w_up, B_w_down):
        any_spec = pl.BlockSpec(memory_space=pl.ANY)
        out = pl.pallas_call(
            kernel,
            out_shape=jax.ShapeDtypeStruct((S, DM), BF16),
            in_specs=[any_spec] * 9,
            out_specs=any_spec,
            scratch_shapes=[
                pltpu.VMEM((NG, DM // 2, GW), U32),
                pltpu.VMEM((NG, DM // 2, GW), U32),
                pltpu.VMEM((NG, DM // 2, GW), U32),
                pltpu.VMEM((H * DH // 2, DM), U32),
                pltpu.VMEM((DM // 2, FF), U32),
                pltpu.VMEM((DM // 2, FF), U32),
                pltpu.VMEM((FF // 2, DM), U32),
                pltpu.VMEM((2, 3, DM, 8, DH), BF16),
                pltpu.VMEM((H * DH, DM), BF16),
                pltpu.VMEM((DM, FF), BF16),
                pltpu.VMEM((DM, FF), BF16),
                pltpu.VMEM((FF, DM), BF16),
                pltpu.VMEM((S, DM), BF16),
                pltpu.VMEM((M, DM), BF16),
                pltpu.VMEM((NP * SEG // 2, DM), U32),
                pltpu.VMEM((R, NG, 3, SEG // 2, GW), U32),
                pltpu.VMEM((2, SEG // 2, DM), U32),
                pltpu.VMEM((MP + 2 * SEG, DM), F32),
                pltpu.VMEM((SEG, DM), F32),
                pltpu.VMEM((XR2, SEG, DM), F32),
                pltpu.VMEM((2, SEG, DM), F32),
                pltpu.VMEM((2, SEG, DM), BF16),
                pltpu.SemaphoreType.DMA((6,)),
                pltpu.SemaphoreType.DMA((7 + WOC,)),
                pltpu.SemaphoreType.DMA((2,)),
            ],
            compiler_params=pltpu.CompilerParams(vmem_limit_bytes=124 * 1024 * 1024),
            name="memtr",
        )(A_x.reshape(S, DM), A_mem0.reshape(M, DM), A_Wq, A_Wk, A_Wv, A_Wo.reshape(H * DH, DM),
          B_w_gate, B_w_up, B_w_down)
        return out.reshape(1, S, DM)
    return run


_run = _make()


@functools.partial(jax.jit, static_argnames=("A_seg_len",))
def pallas_interleave_layers__memory_aug_recurrent_mem_tr__glu_gated_glu__prompt_kernel(
    A_x, A_mem0, A_Wq, A_Wk, A_Wv, A_Wo, A_seg_len, B_x, B_w_gate, B_w_up, B_w_down,
):
    assert A_seg_len == SEG
    assert A_x.shape == (1, S, DM) and A_mem0.shape == (1, M, DM)
    assert A_Wq.shape == (DM, H, DH) and A_Wo.shape == (H, DH, DM)
    assert B_w_gate.shape == (DM, FF) and B_w_down.shape == (FF, DM)
    return _run(A_x, A_mem0, A_Wq, A_Wk, A_Wv, A_Wo, A_seg_len, B_x, B_w_gate, B_w_up, B_w_down)
```
